```python
import jax
import jax.numpy as jnp

def _softmax(x, axis=-1):
    return jax.nn.softmax(x, axis=axis)

def _gelu(x):
    return jax.nn.gelu(x, approximate=True)

def _silu(x):
    return jax.nn.silu(x)

def _sigmoid(x):
    return jax.nn.sigmoid(x)

def _layernorm(x, axis=-1, eps=1e-05):
    m = jnp.mean(x, axis=axis, keepdims=True)
    v = jnp.var(x, axis=axis, keepdims=True)
    return (x - m) / jnp.sqrt(v + eps)

def _scatter_add(tgt, idx, src, axis=0):
    return tgt.at[idx].add(src)

def _segment_sum(src, seg, n):
    return jax.ops.segment_sum(src, seg, n)

class _Rng:

    def __init__(self, key):
        self._k = key

    def _next(self):
        self._k, sub = jax.random.split(self._k)
        return sub

    def normal(self, shape):
        return jax.random.normal(self._next(), shape, dtype=jnp.bfloat16)

    def randint(self, lo, hi, shape):
        return jax.random.randint(self._next(), shape, lo, hi, dtype=jnp.int32)

    def uniform(self, shape, lo=0.0, hi=1.0):
        return jax.random.uniform(self._next(), shape, jnp.bfloat16, lo, hi)

    def permutation(self, n):
        return jax.random.permutation(self._next(), n)
kernel_name = 'adaLN_cond__compressed_kv_cla__dense_activation_relu__decode'

def setup_inputs():
    _rng = _Rng(jax.random.key(int.from_bytes(__import__("os").urandom(4), "little")))
    _w = lambda a: (lambda t: t.astype(jnp.bfloat16) if jnp.issubdtype(t.dtype, jnp.floating) else t)(jnp.asarray(a))

    def _A_setup():
        B, H, Sq, Sk, D, M = (8, 32, 1, 4096, 128, 512)
        Dc = 4 * D
        return {'x': _w((lambda *s: _rng.normal(s) * 0.05)(B, Sq, M)), 'c_kv': _w((lambda *s: _rng.normal(s) * 0.05)(B, Sk, Dc)), 'w_q': _w((lambda *s: _rng.normal(s) * 0.05)(M, H, D) * M ** (-0.5)), 'w_uk': _w((lambda *s: _rng.normal(s) * 0.05)(Dc, H, D) * Dc ** (-0.5)), 'w_uv': _w((lambda *s: _rng.normal(s) * 0.05)(Dc, H, D) * Dc ** (-0.5)), 'w_o': _w((lambda *s: _rng.normal(s) * 0.05)(H, D, M) * (H * D) ** (-0.5))}
    _A_in = _A_setup()

    def _B_setup():
        B, S, D, Dff = (8, 1, 512, 1792)
        return {'x': _w((lambda *s: _rng.normal(s) * 0.05)(B, S, D)), 'w1': _w((lambda *s: _rng.normal(s) * 0.05)(D, Dff)), 'w2': _w((lambda *s: _rng.normal(s) * 0.05)(Dff, D))}
    _B_in = _B_setup()
    return {'A_x': _A_in['x'], 'A_c_kv': _A_in['c_kv'], 'A_w_q': _A_in['w_q'], 'A_w_uk': _A_in['w_uk'], 'A_w_uv': _A_in['w_uv'], 'A_w_o': _A_in['w_o'], 'B_x': _B_in['x'], 'B_w1': _B_in['w1'], 'B_w2': _B_in['w2'], 'c': _w((lambda *s: _rng.normal(s) * 0.05)(8, 512)), 'w_mod': _w((lambda *s: _rng.normal(s) * 0.05)(512, 6 * 512) * 512 ** (-0.5))}

def reference(A_x, A_c_kv, A_w_q, A_w_uk, A_w_uv, A_w_o, B_x, B_w1, B_w2, c, w_mod):

    def _A_ref(x, c_kv, w_q, w_uk, w_uv, w_o):
        B, Sq, M = (x.shape[0], x.shape[1], x.shape[2])
        Sk = c_kv.shape[1]
        H, D = (w_q.shape[1], w_q.shape[2])
        q = jnp.einsum('bqm,mhd->bhqd', x, w_q)
        k = jnp.einsum('bkc,chd->bhkd', c_kv, w_uk)
        v = jnp.einsum('bkc,chd->bhkd', c_kv, w_uv)
        scores = jnp.einsum('bhqd,bhkd->bhqk', q, k) * D ** (-0.5)
        off = Sk - Sq
        qi = jnp.arange(Sq)[:, None]
        kj = jnp.arange(Sk)[None, :]
        cmask = kj <= qi + off
        scores = jnp.where(cmask[None, None], scores, -1000000000.0)
        p = _softmax(scores, axis=-1)
        ctx = jnp.einsum('bhqk,bhkd->bhqd', p, v)
        return jnp.einsum('bhqd,hdm->bqm', ctx, w_o)

    def _B_ref(x, w1, w2):
        h = jnp.einsum('bsd,df->bsf', x, w1)
        zero = jnp.zeros_like(h)
        h = jnp.maximum(h, zero)
        return jnp.einsum('bsf,fd->bsd', h, w2)
    x = A_x
    mod = (_silu(c) @ w_mod).reshape(c.shape[0], 6, 1, -1)
    sa, ca, ga, sb, cb, gb = (mod[:, 0].copy(), mod[:, 1].copy(), mod[:, 2].copy(), mod[:, 3].copy(), mod[:, 4].copy(), mod[:, 5].copy())
    h = _layernorm(x, axis=-1) * (1 + ca) + sa
    x = x + ga * _A_ref(h, A_c_kv, A_w_q, A_w_uk, A_w_uv, A_w_o)
    h = _layernorm(x, axis=-1) * (1 + cb) + sb
    x = x + gb * _B_ref(h, B_w1, B_w2)
    return x
```

```python
import functools

import jax
import jax.numpy as jnp
from jax import lax
import jax.experimental.pallas as pl
import jax.experimental.pallas.tpu as pltpu

F32 = jnp.float32
BF16 = jnp.bfloat16
U32 = jnp.uint32
LANES = 128
EPS = 1e-05

_NT = (((1,), (1,)), ((), ()))


def _layernorm(x):
    m = jnp.mean(x, axis=-1, keepdims=True)
    d = x - m
    v = jnp.mean(d * d, axis=-1, keepdims=True)
    return d / jnp.sqrt(v + EPS)


def _head_pair(w32, pair, rows, n_pairs):
    a = w32[pl.ds(pair, rows // 2, stride=2 * n_pairs), :]
    b = w32[pl.ds(pair + n_pairs, rows // 2, stride=2 * n_pairs), :]
    lo = jnp.uint32(0x0000FFFF)
    hi = jnp.uint32(0xFFFF0000)
    even = (a & lo) | (b << 16)
    odd = (a >> 16) | (b & hi)
    return pltpu.bitcast(even, BF16), pltpu.bitcast(odd, BF16)


def _kernel(x_hbm, ckv_hbm, wq_hbm, wuk_hbm, wuv_hbm, wo_hbm, w1_hbm, w2_hbm,
            c_hbm, wmod_hbm, out_ref,
            x_v, c_v, ckv_v, wq_v, wuk_v, wuv_v, wo_v, w1_v, w2_v, wmod_v,
            q_s, qa_s, cc_s, ctx_s, sems, kv_sems, *, H, depth, compute):
    B, SK, DC = ckv_hbm.shape
    M = c_hbm.shape[1]
    D = LANES
    NP = H // 2
    NC = DC // LANES

    def cols(ref, i0, i1):
        return ref.at[:, pl.ds(i0 * M, (i1 - i0) * M)]

    def words(src, dst):
        return src.bitcast(U32), dst.at[pl.ds(0, src.shape[0] // 2), :]

    head = [(x_hbm, x_v), (c_hbm, c_v),
            (cols(wmod_hbm, 0, 2), cols(wmod_v, 0, 2)),
            words(wq_hbm, wq_v), words(wuk_hbm, wuk_v)]
    tail = [words(wuv_hbm, wuv_v), (wo_hbm, wo_v),
            (cols(wmod_hbm, 2, 5), cols(wmod_v, 2, 5)),
            (w1_hbm, w1_v), (w2_hbm, w2_v),
            (cols(wmod_hbm, 5, 6), cols(wmod_v, 5, 6))]
    cp = [pltpu.make_async_copy(s, d, sems.at[i]) for i, (s, d) in enumerate(head + tail)]
    (cp_x, cp_c, cp_mod0, cp_wq, cp_wuk,
     cp_wuv, cp_wo, cp_mod1, cp_w1, cp_w2, cp_mod2) = cp
    cp_tail = cp[len(head):]

    def cp_kv(b):
        return pltpu.make_async_copy(ckv_hbm.at[b], ckv_v.at[b], kv_sems.at[b])

    cp_mod0.start()
    cp_c.start()
    cp_x.start()
    cp_wq.start()
    cp_c.wait()
    cp_x.wait()
    c = c_v[...].astype(F32)
    sc = (c * jax.nn.sigmoid(c)).astype(BF16)
    x = x_v[...].astype(F32)
    xn = _layernorm(x)
    cp_mod0.wait()
    cp_wuk.start()
    mod0 = jnp.dot(sc, wmod_v[:, 0:2 * M], preferred_element_type=F32)
    h = (xn * (1.0 + mod0[:, M:2 * M]) + mod0[:, 0:M]).astype(BF16)

    cp_wq.wait()
    for b in range(depth - 1):
        cp_kv(b).start()
    wq32 = wq_v

    def q_body(j, carry):
        for r, w in enumerate(_head_pair(wq32, j, M, NP)):
            q_s[2 * j + r] = jnp.dot(h, w, preferred_element_type=F32)
        return carry

    if compute:
        lax.fori_loop(0, NP, q_body, 0)

    cp_wuk.wait()
    cp_kv(depth - 1).start()
    wuk32 = wuk_v

    def qa_body(j, carry):
        for r, w in enumerate(_head_pair(wuk32, j, DC, NP)):
            hh = 2 * j + r
            qa = lax.dot_general(q_s[hh].astype(BF16), w, _NT,
                                 preferred_element_type=F32) * (D ** -0.5)
            row = pl.multiple_of(hh * B, B)
            for cb in range(NC):
                qa_s[cb, pl.ds(row, B), :] = qa[:, cb * LANES:(cb + 1) * LANES]
        return carry

    if compute:
        lax.fori_loop(0, NP, qa_body, 0)

    def attn_body(b, carry):
        cp_kv(b).wait()

        @pl.when(b + depth < B)
        def _():
            cp_kv(b + depth).start()

        for t in range(depth):
            @pl.when(b + depth == B + t)
            def _():
                cp_tail[t].start()

        if compute:
            qa = jnp.concatenate(
                [qa_s[cb, pl.ds(b, H, stride=B), :] for cb in range(NC)], axis=1).astype(BF16)
            s = lax.dot_general(qa, ckv_v[b], _NT, preferred_element_type=F32)
            m = jnp.max(s, axis=-1, keepdims=True)
            p = jnp.exp(s - m)
            l = jnp.sum(p, axis=-1, keepdims=True)
            cc = jnp.dot(p.astype(BF16), ckv_v[b], preferred_element_type=F32) / l
            row = pl.multiple_of(b * H, H)
            for cb in range(NC):
                cc_s[cb, pl.ds(row, H), :] = cc[:, cb * LANES:(cb + 1) * LANES]
        return carry

    lax.fori_loop(0, B, attn_body, 0)

    nxt = [depth]

    def wait_tail(copy):
        copy.wait()
        if nxt[0] < len(cp_tail):
            cp_tail[nxt[0]].start()
            nxt[0] += 1

    wait_tail(cp_wuv)
    wuv32 = wuv_v

    def ctx_body(j, carry):
        for r, w in enumerate(_head_pair(wuv32, j, DC, NP)):
            hh = 2 * j + r
            cc = jnp.concatenate(
                [cc_s[cb, pl.ds(hh, B, stride=H), :] for cb in range(NC)], axis=1).astype(BF16)
            ctx_s[hh] = jnp.dot(cc, w, preferred_element_type=F32)
        return carry

    if compute:
        lax.fori_loop(0, NP, ctx_body, 0)

    wait_tail(cp_wo)
    if compute:
        ctx = jnp.concatenate([ctx_s[hh] for hh in range(H)], axis=1).astype(BF16)
        attn = jnp.dot(ctx, wo_v[...], preferred_element_type=F32)
    else:
        attn = x

    wait_tail(cp_mod1)
    mod1 = jnp.dot(sc, wmod_v[:, 2 * M:5 * M], preferred_element_type=F32)
    x1 = x + mod1[:, 0:M] * attn
    h2 = (_layernorm(x1) * (1.0 + mod1[:, 2 * M:3 * M]) + mod1[:, M:2 * M]).astype(BF16)
    wait_tail(cp_w1)
    f = jnp.maximum(jnp.dot(h2, w1_v[...], preferred_element_type=F32), 0.0).astype(BF16)
    wait_tail(cp_w2)
    y = jnp.dot(f, w2_v[...], preferred_element_type=F32)
    wait_tail(cp_mod2)
    gb = jnp.dot(sc, wmod_v[:, 5 * M:6 * M], preferred_element_type=F32)
    out_ref[...] = (x1 + gb * y).astype(out_ref.dtype)


def _run(A_x, A_c_kv, A_w_q, A_w_uk, A_w_uv, A_w_o, B_x, B_w1, B_w2, c, w_mod,
         depth=2, compute=True):
    del B_x
    B, SQ, M = A_x.shape
    _, SK, DC = A_c_kv.shape
    _, H, D = A_w_q.shape
    assert SQ == 1 and D == LANES
    operands = (A_x.reshape(B, M), A_c_kv,
                A_w_q.reshape(M * H, D), A_w_uk.reshape(DC * H, D),
                A_w_uv.reshape(DC * H, D), A_w_o.reshape(H * D, M),
                B_w1, B_w2, c, w_mod)
    x2, ckv, wq, wuk, wuv, wo, w1, w2, c2, wmod = operands
    vmem = lambda a: pltpu.VMEM(a.shape, a.dtype)
    words = lambda a: pltpu.VMEM((a.shape[0] // 2 + H, a.shape[1]), U32)
    out = pl.pallas_call(
        functools.partial(_kernel, H=H, depth=depth, compute=compute),
        out_shape=jax.ShapeDtypeStruct((B, M), A_x.dtype),
        in_specs=[pl.BlockSpec(memory_space=pltpu.HBM)] * len(operands),
        out_specs=pl.BlockSpec(memory_space=pltpu.VMEM),
        scratch_shapes=[
            vmem(x2), vmem(c2), vmem(ckv), words(wq), words(wuk), words(wuv), vmem(wo),
            vmem(w1), vmem(w2), vmem(wmod),
            pltpu.VMEM((H, B, D), F32),
            pltpu.VMEM((DC // LANES, H * B + B, LANES), F32),
            pltpu.VMEM((DC // LANES, B * H + H, LANES), F32),
            pltpu.VMEM((H, B, D), F32),
            pltpu.SemaphoreType.DMA((11,)),
            pltpu.SemaphoreType.DMA((B,)),
        ],
        compiler_params=pltpu.CompilerParams(vmem_limit_bytes=100 * 1024 * 1024),
    )(*operands)
    return out.reshape(B, SQ, M)


@jax.jit
def pallas_adaLN_cond__compressed_kv_cla__dense_activation_relu__decode_kernel(
    A_x: jax.Array,
    A_c_kv: jax.Array,
    A_w_q: jax.Array,
    A_w_uk: jax.Array,
    A_w_uv: jax.Array,
    A_w_o: jax.Array,
    B_x: jax.Array,
    B_w1: jax.Array,
    B_w2: jax.Array,
    c: jax.Array,
    w_mod: jax.Array,
):
    return _run(A_x, A_c_kv, A_w_q, A_w_uk, A_w_uv, A_w_o, B_x, B_w1, B_w2, c, w_mod)
```

```python
import functools

import jax
import jax.numpy as jnp
from jax import lax
import jax.experimental.pallas as pl
import jax.experimental.pallas.tpu as pltpu

F32 = jnp.float32
BF16 = jnp.bfloat16
U32 = jnp.uint32
LANES = 128
EPS = 1e-05
RING = 16
KB = 256

_NT = (((1,), (1,)), ((), ()))


def _layernorm(x):
    m = jnp.mean(x, axis=-1, keepdims=True)
    d = x - m
    v = jnp.mean(d * d, axis=-1, keepdims=True)
    return d / jnp.sqrt(v + EPS)


class _Stream:
    def __init__(self, segments, sems, depth, enabled=True):
        self.segs, self.sems, self.depth, self.enabled = [], sems, depth, enabled
        first = 0
        for src, dst, rows, small in segments:
            assert src.shape[0] % rows == 0
            n = src.shape[0] // rows
            self.segs.append((first, first + n, src, dst, rows, small))
            first += n
        self.total = first
        self.done = 0

    def end(self, i):
        return self.segs[i][1]

    def _each(self, g, lo, hi, fn):
        if not self.enabled:
            return
        for first, last, src, dst, rows, small in self.segs:
            if hi < first or lo >= last:
                continue
            run = functools.partial(fn, g - first, self.sems.at[g & (RING - 1)],
                                    src, dst, rows, small)
            if first <= lo and hi < last:
                run()
            elif first <= lo:
                pl.when(g < last)(run)
            elif hi < last:
                pl.when(g >= first)(run)
            else:
                pl.when(jnp.logical_and(g >= first, g < last))(run)

    @staticmethod
    def _rows(start, n):
        if not isinstance(start, int):
            start = pl.multiple_of(start, 8)
        return pl.ds(start, n)

    def _start(self, i, sem, src, dst, rows, small):
        for off, n, prio in ((0, small, 0), (small, rows - small, 1)):
            idx = self._rows(i * rows + off, n)
            pltpu.make_async_copy(src.at[idx], dst.at[idx], sem).start(priority=prio)

    def _wait(self, i, sem, src, dst, rows, small):
        buf = dst.at[self._rows(i * rows, rows)]
        pltpu.make_async_copy(buf, buf, sem).wait()

    def begin(self):
        for g in range(self.depth):
            self._each(g, g, g, self._start)

    def _pump(self, g, lo, hi):
        self._each(g, lo, hi, self._wait)
        d = self.depth
        self._each(g + d, lo + d, hi + d, self._start)

    def pump(self):
        self._pump(self.done, self.done, self.done)
        self.done += 1

    def reserve(self, n):
        base = self.done
        self.done += n
        assert self.done <= self.total
        return lambda i: self._pump(base + i, base, base + n - 1)

    def reserve_split(self, n):
        base, d = self.done, self.depth
        self.done += n
        assert self.done <= self.total
        return (lambda i: self._each(base + i, base, base + n - 1, self._wait),
                lambda i: self._each(base + d + i, base + d, base + d + n - 1, self._start))

    def pump_until(self, g):
        n = g - self.done
        if n > 0:
            pump = self.reserve(n)
            lax.fori_loop(0, n, lambda i, c: (pump(i), c)[1], 0)


def _head_pair(w32, pair, rows, n_pairs):
    a = w32[pl.ds(pair, rows // 2, stride=2 * n_pairs), :]
    b = w32[pl.ds(pair + n_pairs, rows // 2, stride=2 * n_pairs), :]
    even = (a & jnp.uint32(0x0000FFFF)) | (b << 16)
    odd = (a >> 16) | (b & jnp.uint32(0xFFFF0000))
    return pltpu.bitcast(even, BF16), pltpu.bitcast(odd, BF16)


def _kernel(x_hbm, ckv_hbm, wq_hbm, wuk_hbm, wuv_hbm, wo_hbm, w1_hbm, w2_hbm,
            c_hbm, wmod_hbm, out_ref,
            x_v, c_v, ckv_v, wq_v, wuk_v, wuv_v, wo_v, w1_v, w2_v, wmod_v,
            mod_s, q_s, qa_s, s_s, cc_s, ctx_s, small_sems, sems,
            *, H, depth, small, w1g, dma, compute):
    B, M = x_hbm.shape
    DC = ckv_hbm.shape[1]
    SK = ckv_hbm.shape[0] // B
    DFF = w1_hbm.shape[1]
    D = LANES
    NP = H // 2
    NC = DC // LANES
    NK = SK // KB

    stream = _Stream([
        (wmod_hbm, wmod_v, 32, 8),
        (wq_hbm.bitcast(U32), wq_v, 256, 2 * small),
        (wuk_hbm.bitcast(U32), wuk_v, 256, 2 * small),
        (ckv_hbm, ckv_v, 128, small),
        (wuv_hbm.bitcast(U32), wuv_v, 256, 2 * small),
        (wo_hbm, wo_v, 128, small),
        (w1_hbm, w1_v, 32, w1g),
        (w2_hbm, w2_v, 128, small),
    ], sems, depth, dma)
    MOD, WQ, WUK, CKV, WUV, WO, W1, W2 = range(8)

    cp_x = pltpu.make_async_copy(x_hbm, x_v, small_sems.at[0])
    cp_c = pltpu.make_async_copy(c_hbm, c_v, small_sems.at[1])
    stream.begin()
    cp_c.start()
    cp_x.start()
    stream.pump_until(stream.end(MOD))
    cp_c.wait()
    cp_x.wait()
    if not compute:
        stream.pump_until(stream.total)
        out_ref[...] = x_v[...]
        return

    c = c_v[...].astype(F32)
    sc = (c * jax.nn.sigmoid(c)).astype(BF16)
    pump = stream.reserve(6)

    def mod_body(i, carry):
        pump(i)
        w = wmod_v[:, pl.ds(pl.multiple_of(i * M, M), M)]
        mod_s[i] = jnp.dot(sc, w, preferred_element_type=F32)
        return carry

    with jax.named_scope("ph_mod"):
        lax.fori_loop(0, 6, mod_body, 0)
    stream.pump()
    h = (_layernorm(x_v[...].astype(F32)) * (1.0 + mod_s[1]) + mod_s[0]).astype(BF16)

    stream.pump_until(stream.end(WQ))
    wait, start = stream.reserve_split(H)

    def q_body(j, carry):
        wait(2 * j)
        wait(2 * j + 1)
        start(2 * j)
        pair = _head_pair(wq_v, j, M, NP)
        start(2 * j + 1)
        for r, w in enumerate(pair):
            q_s[2 * j + r] = jnp.dot(h, w, preferred_element_type=F32)
        return carry

    with jax.named_scope("ph_q"):
        lax.fori_loop(0, NP, q_body, 0)

    stream.pump_until(stream.end(WUK))
    wait, start = stream.reserve_split(H)

    def qa_body(j, carry):
        wait(2 * j)
        wait(2 * j + 1)
        start(2 * j)
        pair = _head_pair(wuk_v, j, DC, NP)
        start(2 * j + 1)
        for r, w in enumerate(pair):
            hh = 2 * j + r
            qa = lax.dot_general(q_s[hh].astype(BF16), w, _NT,
                                 preferred_element_type=F32) * (D ** -0.5)
            row = pl.multiple_of(hh * B, B)
            for cb in range(NC):
                qa_s[cb, pl.ds(row, B), :] = qa[:, cb * LANES:(cb + 1) * LANES]
        return carry

    with jax.named_scope("ph_qa"):
        lax.fori_loop(0, NP, qa_body, 0)

    def keys(b, k):
        return ckv_v[pl.ds(pl.multiple_of((b * NK + k) * KB, KB), KB), :]

    def fold(op, x):
        return functools.reduce(
            op, [x[:, i * LANES:(i + 1) * LANES] for i in range(KB // LANES)])

    def queries(b):
        return jnp.concatenate(
            [qa_s[cb, pl.ds(b, H, stride=B), :] for cb in range(NC)], axis=1).astype(BF16)

    def scores(qa, b, k, mx):
        s = lax.dot_general(qa, keys(b, k), _NT, preferred_element_type=F32)
        s_s[k] = s
        return jnp.maximum(mx, fold(jnp.maximum, s))

    def apply(m, b, k, l, acc):
        p = jnp.exp(s_s[k] - m)
        acc = acc + jnp.dot(p.astype(BF16), keys(b, k), preferred_element_type=F32)
        return l + fold(jnp.add, p), acc

    def finish(b, l, acc):
        cc = acc / jnp.sum(l, axis=-1, keepdims=True)
        row = b * H if isinstance(b, int) else pl.multiple_of(b * H, H)
        for cb in range(NC):
            cc_s[cb, pl.ds(row, H), :] = cc[:, cb * LANES:(cb + 1) * LANES]

    mx0 = jnp.full((H, LANES), -jnp.inf, F32)
    l0 = jnp.zeros((H, LANES), F32)
    acc0 = jnp.zeros((H, DC), F32)

    per_batch = (stream.end(CKV) - stream.end(WUK)) // B
    assert per_batch == 2 * NK
    stream.pump_until(stream.end(WUK) + per_batch)
    pump = stream.reserve(NK)
    qa_first = queries(0)

    def first_body(k, mx):
        pump(k)
        return scores(qa_first, 0, k, mx)

    with jax.named_scope("ph_first"):
        mx = lax.fori_loop(0, NK, first_body, mx0)
    wait, start = stream.reserve_split((B - 1) * 2 * NK)

    def batch_body(b, mx_prev):
        m = jnp.max(mx_prev, axis=-1, keepdims=True)
        qa = queries(b)

        def step(k, carry):
            mx, l, acc = carry
            i = ((b - 1) * NK + k) * 2
            wait(i)
            wait(i + 1)
            start(i)
            l, acc = apply(m, b - 1, k, l, acc)
            start(i + 1)
            return scores(qa, b, k, mx), l, acc

        mx, l, acc = lax.fori_loop(0, NK, step, (mx0, l0, acc0))
        finish(b - 1, l, acc)
        return mx

    with jax.named_scope("ph_batches"):
        mx = lax.fori_loop(1, B, batch_body, mx)
    m_last = jnp.max(mx, axis=-1, keepdims=True)
    pump = stream.reserve(NK)

    def last_body(k, carry):
        pump(k)
        return apply(m_last, B - 1, k, *carry)

    with jax.named_scope("ph_last"):
        finish(B - 1, *lax.fori_loop(0, NK, last_body, (l0, acc0)))

    stream.pump_until(stream.end(WUV))
    wait, start = stream.reserve_split(H)

    def ctx_body(j, carry):
        wait(2 * j)
        wait(2 * j + 1)
        start(2 * j)
        pair = _head_pair(wuv_v, j, DC, NP)
        start(2 * j + 1)
        for r, w in enumerate(pair):
            hh = 2 * j + r
            cc = jnp.concatenate(
                [cc_s[cb, pl.ds(hh, B, stride=H), :] for cb in range(NC)], axis=1).astype(BF16)
            ctx_s[hh] = jnp.dot(cc, w, preferred_element_type=F32)
        return carry

    with jax.named_scope("ph_ctx"):
        lax.fori_loop(0, NP, ctx_body, 0)

    stream.pump_until(stream.end(WO))
    pump = stream.reserve(H // 4)

    def wo_body(j, attn):
        ctx = jnp.concatenate([ctx_s[4 * j + r] for r in range(4)], axis=1).astype(BF16)
        w = wo_v[pl.ds(pl.multiple_of(j * 4 * D, 4 * D), 4 * D), :]
        attn = attn + jnp.dot(ctx, w, preferred_element_type=F32)
        pump(j)
        return attn

    with jax.named_scope("ph_wo"):
        attn = lax.fori_loop(0, H // 4, wo_body, jnp.zeros((B, M), F32))

    x1 = x_v[...].astype(F32) + mod_s[2] * attn
    h2 = (_layernorm(x1) * (1.0 + mod_s[4]) + mod_s[3]).astype(BF16)
    stream.pump_until(stream.end(W1))
    y = jnp.zeros((B, M), F32)
    for i in range(DFF // (2 * LANES)):
        cols = slice(i * 2 * LANES, (i + 1) * 2 * LANES)
        f = jnp.dot(h2, w1_v[:, cols], preferred_element_type=F32)
        f = jnp.maximum(f, 0.0).astype(BF16)
        for t in range(2):
            stream.pump()
            lo = (2 * i + t) * LANES
            y = y + jnp.dot(f[:, t * LANES:(t + 1) * LANES], w2_v[lo:lo + LANES, :],
                            preferred_element_type=F32)
    assert stream.done == stream.total
    out_ref[...] = (x1 + mod_s[5] * y).astype(out_ref.dtype)


def _run(A_x, A_c_kv, A_w_q, A_w_uk, A_w_uv, A_w_o, B_x, B_w1, B_w2, c, w_mod,
         depth=14, small=48, w1g=16, dma=True, compute=True):
    del B_x
    B, SQ, M = A_x.shape
    _, SK, DC = A_c_kv.shape
    _, H, D = A_w_q.shape
    assert SQ == 1 and D == LANES
    operands = (A_x.reshape(B, M), A_c_kv.reshape(B * SK, DC),
                A_w_q.reshape(M * H, D), A_w_uk.reshape(DC * H, D),
                A_w_uv.reshape(DC * H, D), A_w_o.reshape(H * D, M),
                B_w1, B_w2, c, w_mod)
    x2, ckv, wq, wuk, wuv, wo, w1, w2, c2, wmod = operands
    vmem = lambda a: pltpu.VMEM(a.shape, a.dtype)
    words = lambda a: pltpu.VMEM((a.shape[0] // 2 + H, a.shape[1]), U32)
    out = pl.pallas_call(
        functools.partial(_kernel, H=H, depth=depth, small=small, w1g=w1g,
                          dma=dma, compute=compute),
        out_shape=jax.ShapeDtypeStruct((B, M), A_x.dtype),
        in_specs=[pl.BlockSpec(memory_space=pltpu.HBM)] * len(operands),
        out_specs=pl.BlockSpec(memory_space=pltpu.VMEM),
        scratch_shapes=[
            vmem(x2), vmem(c2), vmem(ckv), words(wq), words(wuk), words(wuv), vmem(wo),
            vmem(w1), vmem(w2), vmem(wmod),
            pltpu.VMEM((6, B, M), F32),
            pltpu.VMEM((H, B, D), F32),
            pltpu.VMEM((DC // LANES, H * B + B, LANES), F32),
            pltpu.VMEM((SK // KB, H, KB), F32),
            pltpu.VMEM((DC // LANES, B * H + H, LANES), F32),
            pltpu.VMEM((H, B, D), F32),
            pltpu.SemaphoreType.DMA((2,)),
            pltpu.SemaphoreType.DMA((RING,)),
        ],
        compiler_params=pltpu.CompilerParams(vmem_limit_bytes=100 * 1024 * 1024,
                                             disable_bounds_checks=True),
    )(*operands)
    return out.reshape(B, SQ, M)


@jax.jit
def pallas_adaLN_cond__compressed_kv_cla__dense_activation_relu__decode_kernel(
    A_x: jax.Array,
    A_c_kv: jax.Array,
    A_w_q: jax.Array,
    A_w_uk: jax.Array,
    A_w_uv: jax.Array,
    A_w_o: jax.Array,
    B_x: jax.Array,
    B_w1: jax.Array,
    B_w2: jax.Array,
    c: jax.Array,
    w_mod: jax.Array,
):
    return _run(A_x, A_c_kv, A_w_q, A_w_uk, A_w_uv, A_w_o, B_x, B_w1, B_w2, c, w_mod)
```

```python
import functools

import jax
import jax.numpy as jnp
from jax import lax
import jax.experimental.pallas as pl
import jax.experimental.pallas.tpu as pltpu

F32 = jnp.float32
BF16 = jnp.bfloat16
U32 = jnp.uint32
LANES = 128
EPS = 1e-05
RING = 32
KB = 512

_NT = (((1,), (1,)), ((), ()))


def _layernorm(x):
    m = jnp.mean(x, axis=-1, keepdims=True)
    d = x - m
    v = jnp.mean(d * d, axis=-1, keepdims=True)
    return d / jnp.sqrt(v + EPS)


class _Stream:
    def __init__(self, segments, sems, ahead, enabled=True):
        assert max(ahead) < RING
        self.segs, self.sems, self.ahead, self.enabled = [], sems, ahead, enabled
        first = 0
        for src, dst, rows, small in segments:
            assert src.shape[0] % rows == 0
            n = src.shape[0] // rows
            self.segs.append((first, first + n, src, dst, rows, small))
            first += n
        self.total = first
        self.done = 0

    def end(self, i):
        return self.segs[i][1]

    def _each(self, g, lo, hi, fn):
        if not self.enabled:
            return
        for first, last, src, dst, rows, small in self.segs:
            if hi < first or lo >= last:
                continue
            run = functools.partial(fn, g - first, self.sems.at[g & (RING - 1)],
                                    src, dst, rows, small)
            if first <= lo and hi < last:
                run()
            elif first <= lo:
                pl.when(g < last)(run)
            elif hi < last:
                pl.when(g >= first)(run)
            else:
                pl.when(jnp.logical_and(g >= first, g < last))(run)

    @staticmethod
    def _rows(start, n):
        if not isinstance(start, int):
            start = pl.multiple_of(start, 8)
        return pl.ds(start, n)

    def _start(self, prio, i, sem, src, dst, rows, small):
        off, n = ((0, small), (small, rows - small))[prio]
        idx = self._rows(i * rows + off, n)
        pltpu.make_async_copy(src.at[idx], dst.at[idx], sem).start(priority=prio)

    def _wait(self, i, sem, src, dst, rows, small):
        buf = dst.at[self._rows(i * rows, rows)]
        pltpu.make_async_copy(buf, buf, sem).wait()

    def begin(self):
        for g in range(max(self.ahead)):
            for prio, d in enumerate(self.ahead):
                if g < d:
                    self._each(g, g, g, functools.partial(self._start, prio))

    def reserve(self, n):
        base = self.done
        self.done += n
        assert self.done <= self.total

        def wait(i):
            self._each(base + i, base, base + n - 1, self._wait)

        def start(i):
            for prio, d in enumerate(self.ahead):
                self._each(base + d + i, base + d, base + d + n - 1,
                           functools.partial(self._start, prio))

        return wait, start

    def pumps(self, n):
        wait, start = self.reserve(n)
        return lambda i: (wait(i), start(i))

    def pump(self):
        self.pumps(1)(0)

    def pump_until(self, g):
        n = g - self.done
        if n > 0:
            pump = self.pumps(n)
            lax.fori_loop(0, n, lambda i, c: (pump(i), c)[1], 0)


def _head_pair(w32, pair, rows, n_pairs):
    return pltpu.bitcast(w32[pl.ds(pair, rows, stride=n_pairs), :], BF16)


def _lane_blocks(x, width):
    return [x[:, i:i + width] for i in range(0, x.shape[1], width)]


def _kernel(x_hbm, ckv_hbm, wq_hbm, wuk_hbm, wuv_hbm, wo_hbm, w1_hbm, w2_hbm,
            c_hbm, wmod_hbm, out_ref,
            x_v, c_v, ckv_v, wq_v, wuk_v, wuv_v, wo_v, w1_v, w2_v, wmod_v,
            dup_s, mod_s, q_s, qa_s, s_s, cc_s, ctx_s, y_s, small_sems, sems,
            *, H, ahead, small, w1g, cuts, dma, compute):
    B, M = x_hbm.shape
    DC = ckv_hbm.shape[1]
    SK = ckv_hbm.shape[0] // B
    DFF = w1_hbm.shape[1]
    D = LANES
    NP = H // 2
    NK = SK // KB

    stream = _Stream([
        (wmod_hbm, wmod_v, 32, 8),
        (wq_hbm.bitcast(U32), wq_v, 256, 2 * small),
        (wuk_hbm.bitcast(U32), wuk_v, 256, 2 * small),
        (ckv_hbm, ckv_v, 128, small),
        (wuv_hbm.bitcast(U32), wuv_v, 256, 2 * small),
        (wo_hbm, wo_v, 128, small),
        (w1_hbm, w1_v) + w1g,
        (w2_hbm, w2_v, 128, small),
    ], sems, ahead, dma)
    MOD, WQ, WUK, CKV, WUV, WO, W1, W2 = range(8)

    cp_x = pltpu.make_async_copy(x_hbm, x_v, small_sems.at[0])
    cp_c = pltpu.make_async_copy(c_hbm, c_v, small_sems.at[1])
    stream.begin()
    cp_c.start()
    cp_x.start()

    dup_s[...] = (lax.broadcasted_iota(jnp.int32, dup_s.shape, 0)
                  == lax.broadcasted_iota(jnp.int32, dup_s.shape, 1) >> 1).astype(F32).astype(BF16)

    def duplicate(x):
        return jnp.concatenate(
            [jnp.dot(t, dup_s[...], preferred_element_type=F32)
             for t in _lane_blocks(x.astype(BF16), LANES)], axis=1)

    def own_head(x):
        row = lax.broadcasted_iota(jnp.int32, x.shape, 0)
        lane = lax.broadcasted_iota(jnp.int32, x.shape, 1)
        return jnp.where((row >= B) == ((lane & 1) == 1), x, 0.0)

    stream.pump_until(stream.end(MOD))
    cp_c.wait()
    cp_x.wait()
    if not compute:
        stream.pump_until(stream.total)
        out_ref[...] = x_v[...]
        return

    c = c_v[...].astype(F32)
    sc = (c * jax.nn.sigmoid(c)).astype(BF16)
    pump = stream.pumps(12)

    def mod_body(i, carry):
        w = wmod_v[:, pl.ds(pl.multiple_of(i * M, M), M)]
        mod_s[i] = jnp.dot(sc, w, preferred_element_type=F32)
        pump(2 * i)
        pump(2 * i + 1)
        return carry

    with jax.named_scope("ph_mod"):
        lax.fori_loop(0, 6, mod_body, 0)
    h = _layernorm(x_v[...].astype(F32)) * (1.0 + mod_s[1]) + mod_s[0]
    stream.pump()
    hd = duplicate(h)
    hd = own_head(jnp.concatenate([hd, hd], axis=0)).astype(BF16)

    stream.pump_until(stream.end(WQ))
    pump = stream.pumps(H)

    def q_body(j, carry):
        q_s[j] = jnp.dot(hd, _head_pair(wq_v, j, M, NP), preferred_element_type=F32)
        pump(2 * j)
        pump(2 * j + 1)
        return carry

    with jax.named_scope("ph_q"):
        lax.fori_loop(0, NP, q_body, 0)

    stream.pump_until(stream.end(WUK))
    pump = stream.pumps(H)

    def qa_body(j, carry):
        qa = lax.dot_general(q_s[j].astype(BF16), _head_pair(wuk_v, j, DC, NP), _NT,
                             preferred_element_type=F32)
        row = pl.multiple_of(j * 2 * B, 2 * B)
        for i, t in enumerate(_lane_blocks(own_head(qa * (D ** -0.5)), LANES)):
            qa_s[i, pl.ds(row, 2 * B), :] = t
        pump(2 * j)
        pump(2 * j + 1)
        return carry

    with jax.named_scope("ph_qa"):
        lax.fori_loop(0, NP, qa_body, 0)

    def keys(b, k, part=0, parts=1):
        n = KB // parts
        return ckv_v[pl.ds(pl.multiple_of((b * NK + k) * KB + part * n, n), n), :]

    def fold(op, x):
        return functools.reduce(op, _lane_blocks(x, LANES))

    def queries(b):
        wide = jnp.concatenate(
            [qa_s[i, pl.ds(b, H, stride=B), :] for i in range(qa_s.shape[0])], axis=1)
        return jnp.concatenate(
            [lax.dot_general(t, dup_s[...], _NT, preferred_element_type=F32)
             for t in _lane_blocks(wide.astype(BF16), 2 * LANES)], axis=1).astype(BF16)

    def scores(qa, b, k, part=0, parts=1):
        return lax.dot_general(qa, keys(b, k, part, parts), _NT, preferred_element_type=F32)

    def apply(s, m, b, k, l, acc):
        p = jnp.exp(s - m)
        acc = acc + jnp.dot(p.astype(BF16), keys(b, k), preferred_element_type=F32)
        return l + fold(jnp.add, p), acc

    def finish(b, l, acc):
        cc = duplicate(acc / jnp.sum(l, axis=-1, keepdims=True))
        for i, t in enumerate(_lane_blocks(cc, LANES)):
            cc_s[i, pl.ds(b, H, stride=B), :] = t

    mx0 = jnp.full((H, LANES), -jnp.inf, F32)
    l0 = jnp.zeros((H, LANES), F32)
    acc0 = jnp.zeros((H, DC), F32)

    assert stream.end(CKV) - stream.end(WUK) == 4 * NK * B
    qa_first = queries(0)
    stream.pump_until(stream.end(WUK) + 4 * NK)
    wait, start = stream.reserve(2 * NK)

    def first_body(k, mx):
        wait(2 * k)
        start(2 * k)
        s0 = scores(qa_first, 0, k, 0, 2)
        start(2 * k + 1)
        s = jnp.concatenate([s0, scores(qa_first, 0, k, 1, 2)], axis=1)
        s_s[k] = s
        mx = jnp.maximum(mx, fold(jnp.maximum, s))
        wait(2 * k + 1)
        return mx

    with jax.named_scope("ph_first"):
        mx = lax.fori_loop(0, NK, first_body, mx0)
    wait, start = stream.reserve((B - 1) * 4 * NK)

    def batch_body(b, mx_prev):
        m = jnp.max(mx_prev, axis=-1, keepdims=True)
        qa = queries(b)

        def step(k, carry):
            mx, l, acc = carry
            i = ((b - 1) * NK + k) * 4
            wait(i)
            start(i)
            wait(i + 1)
            start(i + 1)
            s = scores(qa, b, k)
            start(i + 2)
            l, acc = apply(s_s[k], m, b - 1, k, l, acc)
            s_s[k] = s
            mx = jnp.maximum(mx, fold(jnp.maximum, s))
            wait(i + 2)
            wait(i + 3)
            start(i + 3)
            return mx, l, acc

        mx, l, acc = lax.fori_loop(0, NK, step, (mx0, l0, acc0))
        finish(b - 1, l, acc)
        return mx

    with jax.named_scope("ph_batches"):
        mx = lax.fori_loop(1, B, batch_body, mx)
    m_last = jnp.max(mx, axis=-1, keepdims=True)
    pump = stream.pumps(2 * NK)

    def last_body(k, carry):
        carry = apply(s_s[k], m_last, B - 1, k, *carry)
        pump(2 * k)
        pump(2 * k + 1)
        return carry

    with jax.named_scope("ph_last"):
        out = lax.fori_loop(0, NK, last_body, (l0, acc0))
    finish(B - 1, *out)

    stream.pump_until(stream.end(WUV) + 1)
    pump = stream.pumps(H)

    def ctx_body(j, carry):
        row = pl.multiple_of(j * 2 * B, 2 * B)
        cc = jnp.concatenate(
            [cc_s[i, pl.ds(row, 2 * B), :] for i in range(cc_s.shape[0])], axis=1)
        ctx_s[j] = jnp.dot(own_head(cc).astype(BF16), _head_pair(wuv_v, j, DC, NP),
                           preferred_element_type=F32)
        pump(2 * j)
        pump(2 * j + 1)
        return carry

    with jax.named_scope("ph_ctx"):
        lax.fori_loop(0, NP, ctx_body, 0)

    stream.pump_until(stream.end(WO))
    pump = stream.pumps(H // 8)

    def wo_body(j, attn):
        ctx = jnp.concatenate(
            [ctx_s[4 * j + r, t * B:(t + 1) * B, :] for r in range(4) for t in range(2)], axis=1)
        w = wo_v[pl.ds(pl.multiple_of(j * 8 * D, 8 * D), 8 * D), :]
        attn = attn + jnp.dot(ctx.astype(BF16), w, preferred_element_type=F32)
        pump(j)
        return attn

    with jax.named_scope("ph_wo"):
        attn = lax.fori_loop(0, H // 8, wo_body, jnp.zeros((B, M), F32))

    x1 = x_v[...].astype(F32) + mod_s[2] * attn
    h2 = (_layernorm(x1) * (1.0 + mod_s[4]) + mod_s[3]).astype(BF16)
    stream.pump_until(max(stream.end(W1), stream.total - min(ahead)))
    f = jnp.maximum(jnp.dot(h2, w1_v[...], preferred_element_type=F32), 0.0).astype(BF16)
    y_s[...] = x1

    def project(lo, hi):
        stream.pump_until(stream.end(W1) + hi)
        return y_s[...] + mod_s[5] * jnp.dot(
            f[:, lo * LANES:hi * LANES], w2_v[lo * LANES:hi * LANES, :],
            preferred_element_type=F32)

    for lo, hi in zip((0,) + cuts, cuts):
        y_s[...] = project(lo, hi)
    out_ref[...] = project(cuts[-1], DFF // LANES).astype(out_ref.dtype)
    assert stream.done == stream.total


def _run(A_x, A_c_kv, A_w_q, A_w_uk, A_w_uv, A_w_o, B_x, B_w1, B_w2, c, w_mod,
         ahead=(14, 16), small=48, w1g=(64, 16), cuts=(8, 12), dma=True, compute=True, nosem=True):
    del B_x
    B, SQ, M = A_x.shape
    _, SK, DC = A_c_kv.shape
    _, H, D = A_w_q.shape
    assert SQ == 1 and D == LANES
    operands = (A_x.reshape(B, M), A_c_kv.reshape(B * SK, DC),
                A_w_q.reshape(M * H, D), A_w_uk.reshape(DC * H, D),
                A_w_uv.reshape(DC * H, D), A_w_o.reshape(H * D, M),
                B_w1, B_w2, c, w_mod)
    x2, ckv, wq, wuk, wuv, wo, w1, w2, c2, wmod = operands
    vmem = lambda a: pltpu.VMEM(a.shape, a.dtype)
    words = lambda a: pltpu.VMEM((a.shape[0] // 2 + H, a.shape[1]), U32)
    out = pl.pallas_call(
        functools.partial(_kernel, H=H, ahead=ahead, small=small, w1g=w1g, cuts=cuts,
                          dma=dma, compute=compute),
        out_shape=jax.ShapeDtypeStruct((B, M), A_x.dtype),
        in_specs=[pl.BlockSpec(memory_space=pltpu.HBM)] * len(operands),
        out_specs=pl.BlockSpec(memory_space=pltpu.VMEM),
        scratch_shapes=[
            vmem(x2), vmem(c2), vmem(ckv), words(wq), words(wuk), words(wuv), vmem(wo),
            vmem(w1), vmem(w2), vmem(wmod),
            pltpu.VMEM((LANES, 2 * LANES), BF16),
            pltpu.VMEM((6, B, M), F32),
            pltpu.VMEM((H // 2, 2 * B, D), F32),
            pltpu.VMEM((2 * DC // LANES, H * B + B, LANES), F32),
            pltpu.VMEM((SK // KB, H, KB), F32),
            pltpu.VMEM((2 * DC // LANES, H * B + B, LANES), F32),
            pltpu.VMEM((H // 2, 2 * B, D), F32),
            pltpu.VMEM((B, M), F32),
            pltpu.SemaphoreType.DMA((2,)),
            pltpu.SemaphoreType.DMA((RING,)),
        ],
        compiler_params=pltpu.CompilerParams(vmem_limit_bytes=100 * 1024 * 1024,
                                             disable_bounds_checks=True, disable_semaphore_checks=nosem),
    )(*operands)
    return out.reshape(B, SQ, M)


@jax.jit
def pallas_adaLN_cond__compressed_kv_cla__dense_activation_relu__decode_kernel(
    A_x: jax.Array,
    A_c_kv: jax.Array,
    A_w_q: jax.Array,
    A_w_uk: jax.Array,
    A_w_uv: jax.Array,
    A_w_o: jax.Array,
    B_x: jax.Array,
    B_w1: jax.Array,
    B_w2: jax.Array,
    c: jax.Array,
    w_mod: jax.Array,
):
    return _run(A_x, A_c_kv, A_w_q, A_w_uk, A_w_uv, A_w_o, B_x, B_w1, B_w2, c, w_mod)
```

```python
import functools

import jax
import jax.numpy as jnp
from jax import lax
import jax.experimental.pallas as pl
import jax.experimental.pallas.tpu as pltpu

F32 = jnp.float32
BF16 = jnp.bfloat16
U32 = jnp.uint32
LANES = 128
EPS = 1e-05
RING = 32
WG = 256
WPITCH = WG + 8
KB = 512

_NT = (((1,), (1,)), ((), ()))


def _layernorm(x):
    m = jnp.mean(x, axis=-1, keepdims=True)
    d = x - m
    v = jnp.mean(d * d, axis=-1, keepdims=True)
    return d / jnp.sqrt(v + EPS)


class _Stream:
    def __init__(self, segments, sems, ahead, enabled=True):
        assert max(ahead) < RING
        self.segs, self.sems, self.ahead, self.enabled = [], sems, ahead, enabled
        first = 0
        for src, dst, rows, small, pitch in segments:
            assert src.shape[0] % rows == 0
            n = src.shape[0] // rows
            self.segs.append((first, first + n, src, dst, rows, small, pitch))
            first += n
        self.total = first
        self.done = 0

    def end(self, i):
        return self.segs[i][1]

    def _each(self, g, lo, hi, fn):
        if not self.enabled:
            return
        for first, last, *seg in self.segs:
            if hi < first or lo >= last:
                continue
            run = functools.partial(fn, g - first, self.sems.at[g & (RING - 1)], *seg)
            if first <= lo and hi < last:
                run()
            elif first <= lo:
                pl.when(g < last)(run)
            elif hi < last:
                pl.when(g >= first)(run)
            else:
                pl.when(jnp.logical_and(g >= first, g < last))(run)

    @staticmethod
    def _rows(start, n):
        if not isinstance(start, int):
            start = pl.multiple_of(start, 8)
        return pl.ds(start, n)

    def _start(self, prio, i, sem, src, dst, rows, small, pitch):
        off, n = ((0, small), (small, rows - small))[prio]
        pltpu.make_async_copy(src.at[self._rows(i * rows + off, n)],
                              dst.at[self._rows(i * pitch + off, n)],
                              sem).start(priority=prio)

    def _wait(self, i, sem, src, dst, rows, small, pitch):
        buf = dst.at[self._rows(i * pitch, rows)]
        pltpu.make_async_copy(buf, buf, sem).wait()

    def begin(self):
        for g in range(max(self.ahead)):
            for prio, d in enumerate(self.ahead):
                if g < d:
                    self._each(g, g, g, functools.partial(self._start, prio))

    def reserve(self, n):
        base = self.done
        self.done += n
        assert self.done <= self.total

        def wait(i):
            self._each(base + i, base, base + n - 1, self._wait)

        def start(i):
            for prio, d in enumerate(self.ahead):
                self._each(base + d + i, base + d, base + d + n - 1,
                           functools.partial(self._start, prio))

        return wait, start

    def pumps(self, n):
        wait, start = self.reserve(n)
        return lambda i: (wait(i), start(i))

    def pump(self):
        self.pumps(1)(0)

    def pump_until(self, g):
        n = g - self.done
        if n > 0:
            pump = self.pumps(n)
            lax.fori_loop(0, n, lambda i, c: (pump(i), c)[1], 0)


def _head_pair(w32, pair, rows, n_pairs):
    per_group = WG // n_pairs
    words = [w32[pl.ds(blk * 8 * WPITCH + i * n_pairs + pair, 8, stride=WPITCH), :]
             for blk in range(rows // LANES) for i in range(per_group)]
    return pltpu.bitcast(jnp.concatenate(words, axis=0), BF16)


def _lane_blocks(x, width):
    return [x[:, i:i + width] for i in range(0, x.shape[1], width)]


def _kernel(x_hbm, ckv_hbm, wq_hbm, wuk_hbm, wuv_hbm, wo_hbm, w1_hbm, w2_hbm,
            c_hbm, wmod_hbm, out_ref,
            x_v, c_v, ckv_v, wq_v, wuk_v, wuv_v, wo_v, w1_v, w2_v, wmod_v,
            dup_s, mod_s, q_s, qa_s, s_s, cc_s, ctx_s, y_s, small_sems, sems,
            *, H, ahead, small, w1g, cuts, dma, compute):
    B, M = x_hbm.shape
    DC = ckv_hbm.shape[1]
    SK = ckv_hbm.shape[0] // B
    DFF = w1_hbm.shape[1]
    D = LANES
    NP = H // 2
    NK = SK // KB

    stream = _Stream([
        (wmod_hbm, wmod_v, 32, 8, 32),
        (wq_hbm.bitcast(U32), wq_v, WG, 2 * small, WPITCH),
        (wuk_hbm.bitcast(U32), wuk_v, WG, 2 * small, WPITCH),
        (ckv_hbm, ckv_v, 128, small, 128),
        (wuv_hbm.bitcast(U32), wuv_v, WG, 2 * small, WPITCH),
        (wo_hbm, wo_v, 128, small, 128),
        (w1_hbm, w1_v) + w1g,
        (w2_hbm, w2_v, 128, small, 128),
    ], sems, ahead, dma)
    MOD, WQ, WUK, CKV, WUV, WO, W1, W2 = range(8)

    cp_x = pltpu.make_async_copy(x_hbm, x_v, small_sems.at[0])
    cp_c = pltpu.make_async_copy(c_hbm, c_v, small_sems.at[1])
    stream.begin()
    cp_c.start()
    cp_x.start()

    assert (WG // NP) * 8 == LANES
    col = lax.broadcasted_iota(jnp.int32, dup_s.shape, 1) >> 1
    dup_s[...] = (lax.broadcasted_iota(jnp.int32, dup_s.shape, 0)
                  == (col & 7) * (WG // NP) + (col >> 3)).astype(F32).astype(BF16)

    def duplicate(x):
        return jnp.concatenate(
            [jnp.dot(t, dup_s[...], preferred_element_type=F32)
             for t in _lane_blocks(x.astype(BF16), LANES)], axis=1)

    def own_head(x):
        row = lax.broadcasted_iota(jnp.int32, x.shape, 0)
        lane = lax.broadcasted_iota(jnp.int32, x.shape, 1)
        return jnp.where((row >= B) == ((lane & 1) == 1), x, 0.0)

    stream.pump_until(stream.end(MOD))
    cp_c.wait()
    cp_x.wait()
    if not compute:
        stream.pump_until(stream.total)
        out_ref[...] = x_v[...]
        return

    c = c_v[...].astype(F32)
    sc = (c * jax.nn.sigmoid(c)).astype(BF16)
    pump = stream.pumps(12)

    def mod_body(i, carry):
        w = wmod_v[:, pl.ds(pl.multiple_of(i * M, M), M)]
        mod_s[i] = jnp.dot(sc, w, preferred_element_type=F32)
        pump(2 * i)
        pump(2 * i + 1)
        return carry

    with jax.named_scope("ph_mod"):
        lax.fori_loop(0, 6, mod_body, 0)
    h = _layernorm(x_v[...].astype(F32)) * (1.0 + mod_s[1]) + mod_s[0]
    stream.pump()
    hd = duplicate(h)
    hd = own_head(jnp.concatenate([hd, hd], axis=0)).astype(BF16)

    stream.pump_until(stream.end(WQ))
    pump = stream.pumps(H)

    def q_body(j, carry):
        q_s[j] = jnp.dot(hd, _head_pair(wq_v, j, M, NP), preferred_element_type=F32)
        pump(2 * j)
        pump(2 * j + 1)
        return carry

    with jax.named_scope("ph_q"):
        lax.fori_loop(0, NP, q_body, 0)

    stream.pump_until(stream.end(WUK))
    pump = stream.pumps(H)

    def qa_body(j, carry):
        qa = lax.dot_general(q_s[j].astype(BF16), _head_pair(wuk_v, j, DC, NP), _NT,
                             preferred_element_type=F32)
        row = pl.multiple_of(j * 2 * B, 2 * B)
        for i, t in enumerate(_lane_blocks(own_head(qa * (D ** -0.5)), LANES)):
            qa_s[i, pl.ds(row, 2 * B), :] = t
        pump(2 * j)
        pump(2 * j + 1)
        return carry

    with jax.named_scope("ph_qa"):
        lax.fori_loop(0, NP, qa_body, 0)

    def keys(b, k, part=0, parts=1):
        n = KB // parts
        return ckv_v[pl.ds(pl.multiple_of((b * NK + k) * KB + part * n, n), n), :]

    def fold(op, x):
        return functools.reduce(op, _lane_blocks(x, LANES))

    def queries(b):
        wide = jnp.concatenate(
            [qa_s[i, pl.ds(b, H, stride=B), :] for i in range(qa_s.shape[0])], axis=1)
        return jnp.concatenate(
            [lax.dot_general(t, dup_s[...], _NT, preferred_element_type=F32)
             for t in _lane_blocks(wide.astype(BF16), 2 * LANES)], axis=1).astype(BF16)

    def scores(qa, b, k, part=0, parts=1):
        return lax.dot_general(qa, keys(b, k, part, parts), _NT, preferred_element_type=F32)

    def apply(s, m, b, k, l, acc):
        p = jnp.exp(s - m)
        acc = acc + jnp.dot(p.astype(BF16), keys(b, k), preferred_element_type=F32)
        return l + fold(jnp.add, p), acc

    def finish(b, l, acc):
        cc = duplicate(acc / jnp.sum(l, axis=-1, keepdims=True))
        for i, t in enumerate(_lane_blocks(cc, LANES)):
            cc_s[i, pl.ds(b, H, stride=B), :] = t

    mx0 = jnp.full((H, LANES), -jnp.inf, F32)
    l0 = jnp.zeros((H, LANES), F32)
    acc0 = jnp.zeros((H, DC), F32)

    assert stream.end(CKV) - stream.end(WUK) == 4 * NK * B
    qa_first = queries(0)
    stream.pump_until(stream.end(WUK) + 4 * NK)
    wait, start = stream.reserve(2 * NK)

    def first_body(k, mx):
        wait(2 * k)
        start(2 * k)
        s0 = scores(qa_first, 0, k, 0, 2)
        start(2 * k + 1)
        s = jnp.concatenate([s0, scores(qa_first, 0, k, 1, 2)], axis=1)
        s_s[k] = s
        mx = jnp.maximum(mx, fold(jnp.maximum, s))
        wait(2 * k + 1)
        return mx

    with jax.named_scope("ph_first"):
        mx = lax.fori_loop(0, NK, first_body, mx0)
    wait, start = stream.reserve((B - 1) * 4 * NK)

    def batch_body(b, mx_prev):
        m = jnp.max(mx_prev, axis=-1, keepdims=True)
        qa = queries(b)

        def step(k, carry):
            mx, l, acc = carry
            i = ((b - 1) * NK + k) * 4
            wait(i)
            start(i)
            wait(i + 1)
            start(i + 1)
            s = scores(qa, b, k)
            start(i + 2)
            l, acc = apply(s_s[k], m, b - 1, k, l, acc)
            s_s[k] = s
            mx = jnp.maximum(mx, fold(jnp.maximum, s))
            wait(i + 2)
            wait(i + 3)
            start(i + 3)
            return mx, l, acc

        mx, l, acc = lax.fori_loop(0, NK, step, (mx0, l0, acc0))
        finish(b - 1, l, acc)
        return mx

    with jax.named_scope("ph_batches"):
        mx = lax.fori_loop(1, B, batch_body, mx)
    m_last = jnp.max(mx, axis=-1, keepdims=True)
    pump = stream.pumps(2 * NK)

    def last_body(k, carry):
        carry = apply(s_s[k], m_last, B - 1, k, *carry)
        pump(2 * k)
        pump(2 * k + 1)
        return carry

    with jax.named_scope("ph_last"):
        out = lax.fori_loop(0, NK, last_body, (l0, acc0))
    finish(B - 1, *out)

    stream.pump_until(stream.end(WUV) + 1)
    pump = stream.pumps(H)

    def ctx_body(j, carry):
        row = pl.multiple_of(j * 2 * B, 2 * B)
        cc = jnp.concatenate(
            [cc_s[i, pl.ds(row, 2 * B), :] for i in range(cc_s.shape[0])], axis=1)
        ctx_s[j] = jnp.dot(own_head(cc).astype(BF16), _head_pair(wuv_v, j, DC, NP),
                           preferred_element_type=F32)
        pump(2 * j)
        pump(2 * j + 1)
        return carry

    with jax.named_scope("ph_ctx"):
        lax.fori_loop(0, NP, ctx_body, 0)

    stream.pump_until(stream.end(WO))
    pump = stream.pumps(H // 8)

    def wo_body(j, attn):
        ctx = jnp.concatenate(
            [ctx_s[4 * j + r, t * B:(t + 1) * B, :] for r in range(4) for t in range(2)], axis=1)
        w = wo_v[pl.ds(pl.multiple_of(j * 8 * D, 8 * D), 8 * D), :]
        attn = attn + jnp.dot(ctx.astype(BF16), w, preferred_element_type=F32)
        pump(j)
        return attn

    with jax.named_scope("ph_wo"):
        attn = lax.fori_loop(0, H // 8, wo_body, jnp.zeros((B, M), F32))

    x1 = x_v[...].astype(F32) + mod_s[2] * attn
    h2 = (_layernorm(x1) * (1.0 + mod_s[4]) + mod_s[3]).astype(BF16)
    stream.pump_until(max(stream.end(W1), stream.total - min(ahead)))
    f = jnp.maximum(jnp.dot(h2, w1_v[...], preferred_element_type=F32), 0.0).astype(BF16)
    y_s[...] = x1

    def project(lo, hi):
        stream.pump_until(stream.end(W1) + hi)
        return y_s[...] + mod_s[5] * jnp.dot(
            f[:, lo * LANES:hi * LANES], w2_v[lo * LANES:hi * LANES, :],
            preferred_element_type=F32)

    for lo, hi in zip((0,) + cuts, cuts):
        y_s[...] = project(lo, hi)
    out_ref[...] = project(cuts[-1], DFF // LANES).astype(out_ref.dtype)
    assert stream.done == stream.total


def _run(A_x, A_c_kv, A_w_q, A_w_uk, A_w_uv, A_w_o, B_x, B_w1, B_w2, c, w_mod,
         ahead=(14, 16), small=48, w1g=(64, 16, 64), cuts=(8, 12), dma=True, compute=True, nosem=True):
    del B_x
    B, SQ, M = A_x.shape
    _, SK, DC = A_c_kv.shape
    _, H, D = A_w_q.shape
    assert SQ == 1 and D == LANES
    operands = (A_x.reshape(B, M), A_c_kv.reshape(B * SK, DC),
                A_w_q.reshape(M * H, D), A_w_uk.reshape(DC * H, D),
                A_w_uv.reshape(DC * H, D), A_w_o.reshape(H * D, M),
                B_w1, B_w2, c, w_mod)
    x2, ckv, wq, wuk, wuv, wo, w1, w2, c2, wmod = operands
    vmem = lambda a: pltpu.VMEM(a.shape, a.dtype)
    words = lambda a: pltpu.VMEM(((a.shape[0] // 2 // WG + 1) * WPITCH, a.shape[1]), U32)
    out = pl.pallas_call(
        functools.partial(_kernel, H=H, ahead=ahead, small=small, w1g=w1g, cuts=cuts,
                          dma=dma, compute=compute),
        out_shape=jax.ShapeDtypeStruct((B, M), A_x.dtype),
        in_specs=[pl.BlockSpec(memory_space=pltpu.HBM)] * len(operands),
        out_specs=pl.BlockSpec(memory_space=pltpu.VMEM),
        scratch_shapes=[
            vmem(x2), vmem(c2), vmem(ckv), words(wq), words(wuk), words(wuv), vmem(wo),
            vmem(w1), vmem(w2), vmem(wmod),
            pltpu.VMEM((LANES, 2 * LANES), BF16),
            pltpu.VMEM((6, B, M), F32),
            pltpu.VMEM((H // 2, 2 * B, D), F32),
            pltpu.VMEM((2 * DC // LANES, H * B + B, LANES), F32),
            pltpu.VMEM((SK // KB, H, KB), F32),
            pltpu.VMEM((2 * DC // LANES, H * B + B, LANES), F32),
            pltpu.VMEM((H // 2, 2 * B, D), F32),
            pltpu.VMEM((B, M), F32),
            pltpu.SemaphoreType.DMA((2,)),
            pltpu.SemaphoreType.DMA((RING,)),
        ],
        compiler_params=pltpu.CompilerParams(vmem_limit_bytes=100 * 1024 * 1024,
                                             disable_bounds_checks=True, disable_semaphore_checks=nosem),
    )(*operands)
    return out.reshape(B, SQ, M)


@jax.jit
def pallas_adaLN_cond__compressed_kv_cla__dense_activation_relu__decode_kernel(
    A_x: jax.Array,
    A_c_kv: jax.Array,
    A_w_q: jax.Array,
    A_w_uk: jax.Array,
    A_w_uv: jax.Array,
    A_w_o: jax.Array,
    B_x: jax.Array,
    B_w1: jax.Array,
    B_w2: jax.Array,
    c: jax.Array,
    w_mod: jax.Array,
):
    return _run(A_x, A_c_kv, A_w_q, A_w_uk, A_w_uv, A_w_o, B_x, B_w1, B_w2, c, w_mod)
```

```python
import functools

import jax
import jax.numpy as jnp
from jax import lax
import jax.experimental.pallas as pl
import jax.experimental.pallas.tpu as pltpu

F32 = jnp.float32
BF16 = jnp.bfloat16
U32 = jnp.uint32
LANES = 128
EPS = 1e-05
RING = 32
WG = 256
WPITCH = WG + 8
KB = 512

_NT = (((1,), (1,)), ((), ()))


def _layernorm(x):
    m = jnp.mean(x, axis=-1, keepdims=True)
    d = x - m
    v = jnp.mean(d * d, axis=-1, keepdims=True)
    return d / jnp.sqrt(v + EPS)


class _Stream:
    def __init__(self, segments, sems, ahead, enabled=True):
        assert max(ahead) < RING
        self.segs, self.sems, self.ahead, self.enabled = [], sems, ahead, enabled
        first = 0
        for src, dst, rows, small in segments:
            assert src.shape[0] % rows == 0
            n = src.shape[0] // rows
            self.segs.append((first, first + n, src, dst, rows, small))
            first += n
        self.total = first
        self.done = 0

    def end(self, i):
        return self.segs[i][1]

    def _each(self, g, lo, hi, fn):
        if not self.enabled:
            return
        for first, last, *seg in self.segs:
            if hi < first or lo >= last:
                continue
            run = functools.partial(fn, g - first, self.sems.at[g & (RING - 1)], *seg)
            if first <= lo and hi < last:
                run()
            elif first <= lo:
                pl.when(g < last)(run)
            elif hi < last:
                pl.when(g >= first)(run)
            else:
                pl.when(jnp.logical_and(g >= first, g < last))(run)

    @staticmethod
    def _rows(start, n):
        if not isinstance(start, int):
            start = pl.multiple_of(start, 8)
        return pl.ds(start, n)

    def _start(self, prio, i, sem, src, dst, rows, small):
        off, n = ((0, small), (small, rows - small))[prio]
        idx = self._rows(i * rows + off, n)
        pltpu.make_async_copy(src.at[idx], dst.at[idx], sem).start(priority=prio)

    def _wait(self, i, sem, src, dst, rows, small):
        buf = dst.at[self._rows(i * rows, rows)]
        pltpu.make_async_copy(buf, buf, sem).wait()

    def begin(self):
        for g in range(max(self.ahead)):
            for prio, d in enumerate(self.ahead):
                if g < d:
                    self._each(g, g, g, functools.partial(self._start, prio))

    def reserve(self, n):
        base = self.done
        self.done += n
        assert self.done <= self.total

        def wait(i):
            self._each(base + i, base, base + n - 1, self._wait)

        def start(i):
            for prio, d in enumerate(self.ahead):
                self._each(base + d + i, base + d, base + d + n - 1,
                           functools.partial(self._start, prio))

        return wait, start

    def pumps(self, n):
        wait, start = self.reserve(n)
        return lambda i: (wait(i), start(i))

    def pump(self):
        self.pumps(1)(0)

    def pump_until(self, g):
        n = g - self.done
        if n > 0:
            pump = self.pumps(n)
            lax.fori_loop(0, n, lambda i, c: (pump(i), c)[1], 0)


def _to_words(w32, w, g):
    rows = w[pl.ds(pl.multiple_of(g * 2 * WG, 2 * WG), 2 * WG), :]
    w32[pl.ds(pl.multiple_of(g * WPITCH, 8), WG), :] = pltpu.bitcast(rows, U32)


def _head_pair(w32, pair, rows, n_pairs):
    per_group = WG // n_pairs
    words = [w32[pl.ds(blk * 8 * WPITCH + i * n_pairs + pair, 8, stride=WPITCH), :]
             for blk in range(rows // LANES) for i in range(per_group)]
    return pltpu.bitcast(jnp.concatenate(words, axis=0), BF16)


def _lane_blocks(x, width):
    return [x[:, i:i + width] for i in range(0, x.shape[1], width)]


def _kernel(x_hbm, ckv_hbm, wq_hbm, wuk_hbm, wuv_hbm, wo_hbm, w1_hbm, w2_hbm,
            c_hbm, wmod_hbm, out_ref,
            x_v, c_v, ckv_v, wq_v, wuk_v, wuv_v, wo_v, w1_v, w2_v, wmod_v,
            wq_w, wuk_w, wuv_w, dup_s, mod_s, q_s, qa_s, s_s, cc_s, ctx_s, y_s, small_sems, sems,
            *, H, ahead, small, w1g, cuts, dma, compute):
    B, M = x_hbm.shape
    DC = ckv_hbm.shape[1]
    SK = ckv_hbm.shape[0] // B
    DFF = w1_hbm.shape[1]
    D = LANES
    NP = H // 2
    NK = SK // KB

    stream = _Stream([
        (wmod_hbm, wmod_v, 32, 8),
        (wq_hbm, wq_v, 2 * WG, 4 * small),
        (wuk_hbm, wuk_v, 2 * WG, 4 * small),
        (ckv_hbm, ckv_v, 128, small),
        (wuv_hbm, wuv_v, 2 * WG, 4 * small),
        (wo_hbm, wo_v, 128, small),
        (w1_hbm, w1_v) + w1g,
        (w2_hbm, w2_v, 128, small),
    ], sems, ahead, dma)
    MOD, WQ, WUK, CKV, WUV, WO, W1, W2 = range(8)

    cp_x = pltpu.make_async_copy(x_hbm, x_v, small_sems.at[0])
    cp_c = pltpu.make_async_copy(c_hbm, c_v, small_sems.at[1])
    stream.begin()
    cp_c.start()
    cp_x.start()

    assert (WG // NP) * 8 == LANES
    col = lax.broadcasted_iota(jnp.int32, dup_s.shape, 1) >> 1
    dup_s[...] = (lax.broadcasted_iota(jnp.int32, dup_s.shape, 0)
                  == (col & 7) * (WG // NP) + (col >> 3)).astype(F32).astype(BF16)

    def duplicate(x):
        return jnp.concatenate(
            [jnp.dot(t, dup_s[...], preferred_element_type=F32)
             for t in _lane_blocks(x.astype(BF16), LANES)], axis=1)

    def own_head(x):
        row = lax.broadcasted_iota(jnp.int32, x.shape, 0)
        lane = lax.broadcasted_iota(jnp.int32, x.shape, 1)
        return jnp.where((row >= B) == ((lane & 1) == 1), x, 0.0)

    stream.pump_until(stream.end(MOD))
    cp_c.wait()
    cp_x.wait()
    if not compute:
        stream.pump_until(stream.total)
        out_ref[...] = x_v[...]
        return

    c = c_v[...].astype(F32)
    sc = (c * jax.nn.sigmoid(c)).astype(BF16)
    pump = stream.pumps(12)

    def mod_body(i, carry):
        w = wmod_v[:, pl.ds(pl.multiple_of(i * M, M), M)]
        mod_s[i] = jnp.dot(sc, w, preferred_element_type=F32)
        pump(2 * i)
        pump(2 * i + 1)
        return carry

    with jax.named_scope("ph_mod"):
        lax.fori_loop(0, 6, mod_body, 0)
    h = _layernorm(x_v[...].astype(F32)) * (1.0 + mod_s[1]) + mod_s[0]
    stream.pump()
    hd = duplicate(h)
    hd = own_head(jnp.concatenate([hd, hd], axis=0)).astype(BF16)

    stream.pump_until(stream.end(WQ) - NP)
    pump = stream.pumps(NP)

    def wq_body(j, carry):
        pump(j)
        _to_words(wq_w, wq_v, 2 * j)
        _to_words(wq_w, wq_v, 2 * j + 1)
        return carry

    lax.fori_loop(0, NP, wq_body, 0)
    assert stream.done == stream.end(WQ)
    pump = stream.pumps(H)

    def q_body(j, carry):
        q_s[j] = jnp.dot(hd, _head_pair(wq_w, j, M, NP), preferred_element_type=F32)
        for g in (2 * j, 2 * j + 1):
            pump(g)
            _to_words(wuk_w, wuk_v, g)
        return carry

    with jax.named_scope("ph_q"):
        lax.fori_loop(0, NP, q_body, 0)

    stream.pump_until(stream.end(WUK))
    pump = stream.pumps(H)

    def qa_body(j, carry):
        qa = lax.dot_general(q_s[j].astype(BF16), _head_pair(wuk_w, j, DC, NP), _NT,
                             preferred_element_type=F32)
        row = pl.multiple_of(j * 2 * B, 2 * B)
        for i, t in enumerate(_lane_blocks(own_head(qa * (D ** -0.5)), LANES)):
            qa_s[i, pl.ds(row, 2 * B), :] = t
        pump(2 * j)
        pump(2 * j + 1)
        return carry

    with jax.named_scope("ph_qa"):
        lax.fori_loop(0, NP, qa_body, 0)

    def keys(b, k, part=0, parts=1):
        n = KB // parts
        return ckv_v[pl.ds(pl.multiple_of((b * NK + k) * KB + part * n, n), n), :]

    def fold(op, x):
        return functools.reduce(op, _lane_blocks(x, LANES))

    def queries(b):
        wide = jnp.concatenate(
            [qa_s[i, pl.ds(b, H, stride=B), :] for i in range(qa_s.shape[0])], axis=1)
        return jnp.concatenate(
            [lax.dot_general(t, dup_s[...], _NT, preferred_element_type=F32)
             for t in _lane_blocks(wide.astype(BF16), 2 * LANES)], axis=1).astype(BF16)

    def scores(qa, b, k, part=0, parts=1):
        return lax.dot_general(qa, keys(b, k, part, parts), _NT, preferred_element_type=F32)

    def apply(s, m, b, k, l, acc):
        p = jnp.exp(s - m)
        acc = acc + jnp.dot(p.astype(BF16), keys(b, k), preferred_element_type=F32)
        return l + fold(jnp.add, p), acc

    def finish(b, l, acc):
        cc = duplicate(acc / jnp.sum(l, axis=-1, keepdims=True))
        for i, t in enumerate(_lane_blocks(cc, LANES)):
            cc_s[i, pl.ds(b, H, stride=B), :] = t

    mx0 = jnp.full((H, LANES), -jnp.inf, F32)
    l0 = jnp.zeros((H, LANES), F32)
    acc0 = jnp.zeros((H, DC), F32)

    assert stream.end(CKV) - stream.end(WUK) == 4 * NK * B
    qa_first = queries(0)
    stream.pump_until(stream.end(WUK) + 4 * NK)
    wait, start = stream.reserve(2 * NK)

    def first_body(k, mx):
        wait(2 * k)
        start(2 * k)
        s0 = scores(qa_first, 0, k, 0, 2)
        start(2 * k + 1)
        s = jnp.concatenate([s0, scores(qa_first, 0, k, 1, 2)], axis=1)
        s_s[k] = s
        mx = jnp.maximum(mx, fold(jnp.maximum, s))
        wait(2 * k + 1)
        return mx

    with jax.named_scope("ph_first"):
        mx = lax.fori_loop(0, NK, first_body, mx0)
    wait, start = stream.reserve((B - 1) * 4 * NK)

    def batch_body(b, mx_prev):
        m = jnp.max(mx_prev, axis=-1, keepdims=True)
        qa = queries(b)

        def step(k, carry):
            mx, l, acc = carry
            i = ((b - 1) * NK + k) * 4
            wait(i)
            start(i)
            wait(i + 1)
            start(i + 1)
            s = scores(qa, b, k)
            start(i + 2)
            l, acc = apply(s_s[k], m, b - 1, k, l, acc)
            s_s[k] = s
            mx = jnp.maximum(mx, fold(jnp.maximum, s))
            wait(i + 2)
            wait(i + 3)
            start(i + 3)
            return mx, l, acc

        mx, l, acc = lax.fori_loop(0, NK, step, (mx0, l0, acc0))
        finish(b - 1, l, acc)
        return mx

    with jax.named_scope("ph_batches"):
        mx = lax.fori_loop(1, B, batch_body, mx)
    m_last = jnp.max(mx, axis=-1, keepdims=True)
    pump = stream.pumps(2 * NK)

    def last_body(k, carry):
        carry = apply(s_s[k], m_last, B - 1, k, *carry)
        pump(2 * k)
        for g in range(3):
            _to_words(wuv_w, wuv_v, 4 * k + g)
        pump(2 * k + 1)
        _to_words(wuv_w, wuv_v, 4 * k + 3)
        return carry

    with jax.named_scope("ph_last"):
        out = lax.fori_loop(0, NK, last_body, (l0, acc0))
    assert stream.done == stream.end(WUV)
    finish(B - 1, *out)

    stream.pump_until(stream.end(WUV) + 1)
    pump = stream.pumps(H)

    def ctx_body(j, carry):
        row = pl.multiple_of(j * 2 * B, 2 * B)
        cc = jnp.concatenate(
            [cc_s[i, pl.ds(row, 2 * B), :] for i in range(cc_s.shape[0])], axis=1)
        ctx_s[j] = jnp.dot(own_head(cc).astype(BF16), _head_pair(wuv_w, j, DC, NP),
                           preferred_element_type=F32)
        pump(2 * j)
        pump(2 * j + 1)
        return carry

    with jax.named_scope("ph_ctx"):
        lax.fori_loop(0, NP, ctx_body, 0)

    stream.pump_until(stream.end(WO))
    pump = stream.pumps(H // 8)

    def wo_body(j, attn):
        ctx = jnp.concatenate(
            [ctx_s[4 * j + r, t * B:(t + 1) * B, :] for r in range(4) for t in range(2)], axis=1)
        w = wo_v[pl.ds(pl.multiple_of(j * 8 * D, 8 * D), 8 * D), :]
        attn = attn + jnp.dot(ctx.astype(BF16), w, preferred_element_type=F32)
        pump(j)
        return attn

    with jax.named_scope("ph_wo"):
        attn = lax.fori_loop(0, H // 8, wo_body, jnp.zeros((B, M), F32))

    x1 = x_v[...].astype(F32) + mod_s[2] * attn
    h2 = (_layernorm(x1) * (1.0 + mod_s[4]) + mod_s[3]).astype(BF16)
    stream.pump_until(max(stream.end(W1), stream.total - min(ahead)))
    f = jnp.maximum(jnp.dot(h2, w1_v[...], preferred_element_type=F32), 0.0).astype(BF16)
    y_s[...] = x1

    def project(lo, hi):
        stream.pump_until(stream.end(W1) + hi)
        return y_s[...] + mod_s[5] * jnp.dot(
            f[:, lo * LANES:hi * LANES], w2_v[lo * LANES:hi * LANES, :],
            preferred_element_type=F32)

    for lo, hi in zip((0,) + cuts, cuts):
        y_s[...] = project(lo, hi)
    out_ref[...] = project(cuts[-1], DFF // LANES).astype(out_ref.dtype)
    assert stream.done == stream.total


def _run(A_x, A_c_kv, A_w_q, A_w_uk, A_w_uv, A_w_o, B_x, B_w1, B_w2, c, w_mod,
         ahead=(14, 16), small=48, w1g=(64, 16), cuts=(8, 12), dma=True, compute=True, nosem=True, interpret=False):
    del B_x
    B, SQ, M = A_x.shape
    _, SK, DC = A_c_kv.shape
    _, H, D = A_w_q.shape
    assert SQ == 1 and D == LANES
    operands = (A_x.reshape(B, M), A_c_kv.reshape(B * SK, DC),
                A_w_q.reshape(M * H, D), A_w_uk.reshape(DC * H, D),
                A_w_uv.reshape(DC * H, D), A_w_o.reshape(H * D, M),
                B_w1, B_w2, c, w_mod)
    x2, ckv, wq, wuk, wuv, wo, w1, w2, c2, wmod = operands
    vmem = lambda a: pltpu.VMEM(a.shape, a.dtype)
    words = lambda a: pltpu.VMEM(((a.shape[0] // 2 // WG + 1) * WPITCH, a.shape[1]), U32)
    out = pl.pallas_call(
        functools.partial(_kernel, H=H, ahead=ahead, small=small, w1g=w1g, cuts=cuts,
                          dma=dma, compute=compute),
        out_shape=jax.ShapeDtypeStruct((B, M), A_x.dtype),
        in_specs=[pl.BlockSpec(memory_space=pltpu.HBM)] * len(operands),
        out_specs=pl.BlockSpec(memory_space=pltpu.VMEM),
        scratch_shapes=[
            vmem(x2), vmem(c2), vmem(ckv), vmem(wq), vmem(wuk), vmem(wuv), vmem(wo),
            vmem(w1), vmem(w2), vmem(wmod), words(wq), words(wuk), words(wuv),
            pltpu.VMEM((LANES, 2 * LANES), BF16),
            pltpu.VMEM((6, B, M), F32),
            pltpu.VMEM((H // 2, 2 * B, D), F32),
            pltpu.VMEM((2 * DC // LANES, H * B + B, LANES), F32),
            pltpu.VMEM((SK // KB, H, KB), F32),
            pltpu.VMEM((2 * DC // LANES, H * B + B, LANES), F32),
            pltpu.VMEM((H // 2, 2 * B, D), F32),
            pltpu.VMEM((B, M), F32),
            pltpu.SemaphoreType.DMA((2,)),
            pltpu.SemaphoreType.DMA((RING,)),
        ],
        compiler_params=pltpu.CompilerParams(vmem_limit_bytes=100 * 1024 * 1024,
                                             disable_bounds_checks=True, disable_semaphore_checks=nosem),
        interpret=interpret,
    )(*operands)
    return out.reshape(B, SQ, M)


@jax.jit
def pallas_adaLN_cond__compressed_kv_cla__dense_activation_relu__decode_kernel(
    A_x: jax.Array,
    A_c_kv: jax.Array,
    A_w_q: jax.Array,
    A_w_uk: jax.Array,
    A_w_uv: jax.Array,
    A_w_o: jax.Array,
    B_x: jax.Array,
    B_w1: jax.Array,
    B_w2: jax.Array,
    c: jax.Array,
    w_mod: jax.Array,
):
    return _run(A_x, A_c_kv, A_w_q, A_w_uk, A_w_uv, A_w_o, B_x, B_w1, B_w2, c, w_mod)
```

```python
import functools

import jax
import jax.numpy as jnp
from jax import lax
import jax.experimental.pallas as pl
import jax.experimental.pallas.tpu as pltpu

F32 = jnp.float32
BF16 = jnp.bfloat16
U32 = jnp.uint32
LANES = 128
EPS = 1e-05

AHEAD = 14
RING = 16
KB = 512
WG = 256
WPITCH = WG + 8
W2_CUTS = (8, 12)

_NT = (((1,), (1,)), ((), ()))


class _Stream:
    def __init__(self, segments, sems):
        self.segs, self.sems = [], sems
        first = 0
        for src, dst, rows, lead in segments:
            assert src.shape[0] % rows == 0 and rows % 8 == 0 and lead % 8 == 0
            last = first + src.shape[0] // rows
            self.segs.append((first, last, src, dst, rows, lead))
            first = last
        self.total = first
        self.done = 0

    def end(self, segment):
        return self.segs[segment][1]

    def _each(self, g, lo, hi, fn):
        for first, last, *seg in self.segs:
            if hi < first or lo >= last:
                continue
            run = functools.partial(fn, g - first, self.sems.at[g & (RING - 1)], *seg)
            if first <= lo and hi < last:
                run()
            elif first <= lo:
                pl.when(g < last)(run)
            elif hi < last:
                pl.when(g >= first)(run)
            else:
                pl.when(jnp.logical_and(g >= first, g < last))(run)

    @staticmethod
    def _rows(start, n):
        return pl.ds(start if isinstance(start, int) else pl.multiple_of(start, 8), n)

    def _start(self, i, sem, src, dst, rows, lead):
        for priority, (off, n) in enumerate(((0, lead), (lead, rows - lead))):
            idx = self._rows(i * rows + off, n)
            pltpu.make_async_copy(src.at[idx], dst.at[idx], sem).start(priority=priority)

    def _wait(self, i, sem, src, dst, rows, lead):
        buf = dst.at[self._rows(i * rows, rows)]
        pltpu.make_async_copy(buf, buf, sem).wait()

    def begin(self):
        for g in range(AHEAD):
            self._each(g, g, g, self._start)

    def reserve(self, n):
        lo, hi = self.done, self.done + n - 1
        self.done += n
        assert self.done <= self.total
        return (lambda i: self._each(lo + i, lo, hi, self._wait),
                lambda i: self._each(lo + AHEAD + i, lo + AHEAD, hi + AHEAD, self._start))

    def pumps(self, n):
        wait, start = self.reserve(n)

        def pump(i):
            wait(i)
            start(i)

        return pump

    def pump_until(self, g):
        n = g - self.done
        if n == 1:
            self.pumps(1)(0)
        elif n > 1:
            pl.loop(0, n)(self.pumps(n))


def _layernorm(x):
    m = jnp.mean(x, axis=-1, keepdims=True)
    d = x - m
    v = jnp.mean(d * d, axis=-1, keepdims=True)
    return d / jnp.sqrt(v + EPS)


def _lane_blocks(x, width):
    return [x[:, i:i + width] for i in range(0, x.shape[1], width)]


def _to_words(w32, w, g):
    rows = w[pl.ds(pl.multiple_of(g * 2 * WG, 2 * WG), 2 * WG), :]
    w32[pl.ds(pl.multiple_of(g * WPITCH, 8), WG), :] = pltpu.bitcast(rows, U32)


def _head_pair(w32, pair, rows, n_pairs):
    words = [w32[pl.ds(blk * 8 * WPITCH + i * n_pairs + pair, 8, stride=WPITCH), :]
             for blk in range(rows // LANES) for i in range(WG // n_pairs)]
    return pltpu.bitcast(jnp.concatenate(words, axis=0), BF16)


def _kernel(x_hbm, ckv_hbm, wq_hbm, wuk_hbm, wuv_hbm, wo_hbm, w1_hbm, w2_hbm, c_hbm, wmod_hbm,
            out_ref,
            x_v, ckv_v, wq_v, wuk_v, wuv_v, wo_v, w1_v, w2_v, c_v, wmod_v,
            wq_w, wuk_w, wuv_w, dup_s, mod_s, q_s, qa_s, s_s, cc_s, ctx_s, y_s,
            small_sems, sems, *, H):
    B, M = x_hbm.shape
    DC = ckv_hbm.shape[1]
    DFF = w1_hbm.shape[1]
    D = LANES
    NP = H // 2
    NK = ckv_hbm.shape[0] // B // KB

    stream = _Stream([
        (wmod_hbm, wmod_v, 32, 8),
        (wq_hbm, wq_v, 2 * WG, 192),
        (wuk_hbm, wuk_v, 2 * WG, 192),
        (ckv_hbm, ckv_v, KB // 4, 48),
        (wuv_hbm, wuv_v, 2 * WG, 192),
        (wo_hbm, wo_v, LANES, 48),
        (w1_hbm, w1_v, 64, 16),
        (w2_hbm, w2_v, LANES, 48),
    ], sems)
    MOD, WQ, WUK, CKV, WUV, WO, W1 = range(7)
    assert all(stream.end(s) - stream.end(s - 1) == H for s in (WQ, WUK, WUV))
    assert (WG // NP) * 8 == LANES and 4 * NK == H

    cp_x = pltpu.make_async_copy(x_hbm, x_v, small_sems.at[0])
    cp_c = pltpu.make_async_copy(c_hbm, c_v, small_sems.at[1])
    stream.begin()
    cp_c.start()
    cp_x.start()

    col = lax.broadcasted_iota(jnp.int32, dup_s.shape, 1) >> 1
    dup_s[...] = (lax.broadcasted_iota(jnp.int32, dup_s.shape, 0)
                  == (col & 7) * (WG // NP) + (col >> 3)).astype(F32).astype(BF16)

    def duplicate(x):
        return jnp.concatenate(
            [jnp.dot(t, dup_s[...], preferred_element_type=F32)
             for t in _lane_blocks(x.astype(BF16), LANES)], axis=1)

    def own_head(x):
        row = lax.broadcasted_iota(jnp.int32, x.shape, 0)
        lane = lax.broadcasted_iota(jnp.int32, x.shape, 1)
        return jnp.where((row >= B) == ((lane & 1) == 1), x, 0.0)

    stream.pump_until(stream.end(MOD))
    cp_c.wait()
    cp_x.wait()
    c = c_v[...].astype(F32)
    sc = (c * jax.nn.sigmoid(c)).astype(BF16)
    pump = stream.pumps(12)

    @pl.loop(0, 6)
    def _(i):
        w = wmod_v[:, pl.ds(pl.multiple_of(i * M, M), M)]
        mod_s[i] = jnp.dot(sc, w, preferred_element_type=F32)
        pump(2 * i)
        pump(2 * i + 1)

    h = _layernorm(x_v[...].astype(F32)) * (1.0 + mod_s[1]) + mod_s[0]
    stream.pump_until(stream.done + 1)
    hd = duplicate(h)
    hd = own_head(jnp.concatenate([hd, hd], axis=0)).astype(BF16)

    stream.pump_until(stream.end(WQ) - NP)
    pump = stream.pumps(NP)

    @pl.loop(0, NP)
    def _(j):
        pump(j)
        _to_words(wq_w, wq_v, 2 * j)
        _to_words(wq_w, wq_v, 2 * j + 1)

    assert stream.done == stream.end(WQ)
    pump = stream.pumps(H)

    @pl.loop(0, NP)
    def _(j):
        q_s[j] = jnp.dot(hd, _head_pair(wq_w, j, M, NP), preferred_element_type=F32)
        for g in (2 * j, 2 * j + 1):
            pump(g)
            _to_words(wuk_w, wuk_v, g)

    pump = stream.pumps(H)

    @pl.loop(0, NP)
    def _(j):
        qa = lax.dot_general(q_s[j].astype(BF16), _head_pair(wuk_w, j, DC, NP), _NT,
                             preferred_element_type=F32)
        row = pl.multiple_of(j * 2 * B, 2 * B)
        for i, t in enumerate(_lane_blocks(own_head(qa * (D ** -0.5)), LANES)):
            qa_s[i, pl.ds(row, 2 * B), :] = t
        pump(2 * j)
        pump(2 * j + 1)

    def keys(b, k, part=0, parts=1):
        n = KB // parts
        return ckv_v[pl.ds(pl.multiple_of((b * NK + k) * KB + part * n, n), n), :]

    def fold(op, x):
        return functools.reduce(op, _lane_blocks(x, LANES))

    def queries(b):
        wide = jnp.concatenate(
            [qa_s[i, pl.ds(b, H, stride=B), :] for i in range(qa_s.shape[0])], axis=1)
        return jnp.concatenate(
            [lax.dot_general(t, dup_s[...], _NT, preferred_element_type=F32)
             for t in _lane_blocks(wide.astype(BF16), 2 * LANES)], axis=1).astype(BF16)

    def scores(qa, b, k, part=0, parts=1):
        return lax.dot_general(qa, keys(b, k, part, parts), _NT, preferred_element_type=F32)

    def apply(m, b, k, l, acc):
        p = jnp.exp(s_s[k] - m)
        acc = acc + jnp.dot(p.astype(BF16), keys(b, k), preferred_element_type=F32)
        return l + fold(jnp.add, p), acc

    def finish(b, l, acc):
        cc = duplicate(acc / jnp.sum(l, axis=-1, keepdims=True))
        for i, t in enumerate(_lane_blocks(cc, LANES)):
            cc_s[i, pl.ds(b, H, stride=B), :] = t

    mx0 = jnp.full((H, LANES), -jnp.inf, F32)
    l0 = jnp.zeros((H, LANES), F32)
    acc0 = jnp.zeros((H, DC), F32)

    assert stream.done == stream.end(WUK) + 4 * NK
    qa_first = queries(0)
    wait, start = stream.reserve(2 * NK)

    def first_body(k, mx):
        wait(2 * k)
        start(2 * k)
        s0 = scores(qa_first, 0, k, 0, 2)
        start(2 * k + 1)
        s = jnp.concatenate([s0, scores(qa_first, 0, k, 1, 2)], axis=1)
        s_s[k] = s
        mx = jnp.maximum(mx, fold(jnp.maximum, s))
        wait(2 * k + 1)
        return mx

    mx = lax.fori_loop(0, NK, first_body, mx0)
    wait, start = stream.reserve((B - 1) * 4 * NK)

    def batch_body(b, mx_prev):
        m = jnp.max(mx_prev, axis=-1, keepdims=True)
        qa = queries(b)

        def step(k, carry):
            mx, l, acc = carry
            i = ((b - 1) * NK + k) * 4
            wait(i)
            start(i)
            wait(i + 1)
            start(i + 1)
            s = scores(qa, b, k)
            start(i + 2)
            l, acc = apply(m, b - 1, k, l, acc)
            s_s[k] = s
            mx = jnp.maximum(mx, fold(jnp.maximum, s))
            wait(i + 2)
            wait(i + 3)
            start(i + 3)
            return mx, l, acc

        mx, l, acc = lax.fori_loop(0, NK, step, (mx0, l0, acc0))
        finish(b - 1, l, acc)
        return mx

    mx = lax.fori_loop(1, B, batch_body, mx)
    m_last = jnp.max(mx, axis=-1, keepdims=True)
    pump = stream.pumps(2 * NK)

    def last_body(k, carry):
        carry = apply(m_last, B - 1, k, *carry)
        pump(2 * k)
        for g in range(3):
            _to_words(wuv_w, wuv_v, 4 * k + g)
        pump(2 * k + 1)
        _to_words(wuv_w, wuv_v, 4 * k + 3)
        return carry

    finish(B - 1, *lax.fori_loop(0, NK, last_body, (l0, acc0)))
    assert stream.done == stream.end(WUV)

    stream.pump_until(stream.done + 1)
    pump = stream.pumps(H)

    @pl.loop(0, NP)
    def _(j):
        row = pl.multiple_of(j * 2 * B, 2 * B)
        cc = jnp.concatenate(
            [cc_s[i, pl.ds(row, 2 * B), :] for i in range(cc_s.shape[0])], axis=1)
        ctx_s[j] = jnp.dot(own_head(cc).astype(BF16), _head_pair(wuv_w, j, DC, NP),
                           preferred_element_type=F32)
        pump(2 * j)
        pump(2 * j + 1)

    stream.pump_until(stream.end(WO))
    pump = stream.pumps(H // 8)

    def wo_body(j, attn):
        ctx = jnp.concatenate(
            [ctx_s[4 * j + r, t * B:(t + 1) * B, :] for r in range(4) for t in range(2)], axis=1)
        w = wo_v[pl.ds(pl.multiple_of(j * 8 * D, 8 * D), 8 * D), :]
        attn = attn + jnp.dot(ctx.astype(BF16), w, preferred_element_type=F32)
        pump(j)
        return attn

    attn = lax.fori_loop(0, H // 8, wo_body, jnp.zeros((B, M), F32))

    x1 = x_v[...].astype(F32) + mod_s[2] * attn
    h2 = (_layernorm(x1) * (1.0 + mod_s[4]) + mod_s[3]).astype(BF16)
    stream.pump_until(stream.end(W1))
    f = jnp.maximum(jnp.dot(h2, w1_v[...], preferred_element_type=F32), 0.0).astype(BF16)
    y_s[...] = x1

    def project(lo, hi):
        stream.pump_until(stream.end(W1) + hi)
        return y_s[...] + mod_s[5] * jnp.dot(
            f[:, lo * LANES:hi * LANES], w2_v[lo * LANES:hi * LANES, :],
            preferred_element_type=F32)

    for lo, hi in zip((0,) + W2_CUTS, W2_CUTS):
        y_s[...] = project(lo, hi)
    out_ref[...] = project(W2_CUTS[-1], DFF // LANES).astype(out_ref.dtype)
    assert stream.done == stream.total


@jax.jit
def pallas_adaLN_cond__compressed_kv_cla__dense_activation_relu__decode_kernel(
    A_x: jax.Array,
    A_c_kv: jax.Array,
    A_w_q: jax.Array,
    A_w_uk: jax.Array,
    A_w_uv: jax.Array,
    A_w_o: jax.Array,
    B_x: jax.Array,
    B_w1: jax.Array,
    B_w2: jax.Array,
    c: jax.Array,
    w_mod: jax.Array,
):
    del B_x
    B, SQ, M = A_x.shape
    _, SK, DC = A_c_kv.shape
    _, H, D = A_w_q.shape
    assert SQ == 1 and D == LANES
    operands = (A_x.reshape(B, M), A_c_kv.reshape(B * SK, DC),
                A_w_q.reshape(M * H, D), A_w_uk.reshape(DC * H, D), A_w_uv.reshape(DC * H, D),
                A_w_o.reshape(H * D, M), B_w1, B_w2, c, w_mod)
    words = [pltpu.VMEM(((w.shape[0] // (2 * WG) + 1) * WPITCH, D), U32) for w in operands[2:5]]
    out = pl.pallas_call(
        functools.partial(_kernel, H=H),
        out_shape=jax.ShapeDtypeStruct((B, M), A_x.dtype),
        in_specs=[pl.BlockSpec(memory_space=pltpu.HBM)] * len(operands),
        out_specs=pl.BlockSpec(memory_space=pltpu.VMEM),
        scratch_shapes=[pltpu.VMEM(a.shape, a.dtype) for a in operands] + words + [
            pltpu.VMEM((LANES, 2 * LANES), BF16),
            pltpu.VMEM((6, B, M), F32),
            pltpu.VMEM((H // 2, 2 * B, D), F32),
            pltpu.VMEM((2 * DC // LANES, (H + 1) * B, LANES), F32),
            pltpu.VMEM((SK // KB, H, KB), F32),
            pltpu.VMEM((2 * DC // LANES, (H + 1) * B, LANES), F32),
            pltpu.VMEM((H // 2, 2 * B, D), F32),
            pltpu.VMEM((B, M), F32),
            pltpu.SemaphoreType.DMA((2,)),
            pltpu.SemaphoreType.DMA((RING,)),
        ],
        compiler_params=pltpu.CompilerParams(
            vmem_limit_bytes=100 * 1024 * 1024,
            disable_bounds_checks=True,
            disable_semaphore_checks=True,
        ),
    )(*operands)
    return out.reshape(B, SQ, M)
```

```python
import functools

import jax
import jax.numpy as jnp
from jax import lax
import jax.experimental.pallas as pl
import jax.experimental.pallas.tpu as pltpu

F32 = jnp.float32
BF16 = jnp.bfloat16
U32 = jnp.uint32
LANES = 128
EPS = 1e-05

AHEAD = 14
RING = 16
KB = 512
WG = 256
WPITCH = WG + 8
W2_CUTS = (8, 12)

_NT = (((1,), (1,)), ((), ()))


class _Stream:
    def __init__(self, segments, sems):
        self.segs, self.sems = [], sems
        first = 0
        for src, dst, rows, lead in segments:
            assert src.shape[0] % rows == 0 and rows % 8 == 0 and lead % 8 == 0
            last = first + src.shape[0] // rows
            self.segs.append((first, last, src, dst, rows, lead))
            first = last
        self.total = first
        self.done = 0

    def end(self, segment):
        return self.segs[segment][1]

    def _each(self, g, lo, hi, fn):
        for first, last, *seg in self.segs:
            if hi < first or lo >= last:
                continue
            run = functools.partial(fn, g - first, self.sems.at[g & (RING - 1)], *seg)
            if first <= lo and hi < last:
                run()
            elif first <= lo:
                pl.when(g < last)(run)
            elif hi < last:
                pl.when(g >= first)(run)
            else:
                pl.when(jnp.logical_and(g >= first, g < last))(run)

    @staticmethod
    def _rows(start, n):
        return pl.ds(start if isinstance(start, int) else pl.multiple_of(start, 8), n)

    def _start(self, i, sem, src, dst, rows, lead):
        for priority, (off, n) in enumerate(((0, lead), (lead, rows - lead))):
            idx = self._rows(i * rows + off, n)
            pltpu.make_async_copy(src.at[idx], dst.at[idx], sem).start(priority=priority)

    def _wait(self, i, sem, src, dst, rows, lead):
        buf = dst.at[self._rows(i * rows, rows)]
        pltpu.make_async_copy(buf, buf, sem).wait()

    def begin(self):
        for g in range(AHEAD):
            self._each(g, g, g, self._start)

    def reserve(self, n):
        lo, hi = self.done, self.done + n - 1
        self.done += n
        assert self.done <= self.total
        return (lambda i: self._each(lo + i, lo, hi, self._wait),
                lambda i: self._each(lo + AHEAD + i, lo + AHEAD, hi + AHEAD, self._start))

    def pumps(self, n):
        wait, start = self.reserve(n)

        def pump(i):
            wait(i)
            start(i)

        return pump

    def pump_until(self, g):
        n = g - self.done
        if n == 1:
            self.pumps(1)(0)
        elif n > 1:
            pl.loop(0, n)(self.pumps(n))


def _layernorm(x):
    m = jnp.mean(x, axis=-1, keepdims=True)
    d = x - m
    v = jnp.mean(d * d, axis=-1, keepdims=True)
    return d / jnp.sqrt(v + EPS)


def _lane_blocks(x, width):
    return [x[:, i:i + width] for i in range(0, x.shape[1], width)]


def _to_words(w32, w, g):
    rows = w[pl.ds(pl.multiple_of(g * 2 * WG, 2 * WG), 2 * WG), :]
    w32[pl.ds(pl.multiple_of(g * WPITCH, 8), WG), :] = pltpu.bitcast(rows, U32)


def _head_pair(w32, pair, rows, n_pairs):
    words = [w32[pl.ds(blk * 8 * WPITCH + i * n_pairs + pair, 8, stride=WPITCH), :]
             for blk in range(rows // LANES) for i in range(WG // n_pairs)]
    return pltpu.bitcast(jnp.concatenate(words, axis=0), BF16)


def _kernel(x_hbm, ckv_hbm, wq_hbm, wuk_hbm, wuv_hbm, wo_hbm, w1_hbm, w2_hbm, c_hbm, wmod_hbm,
            out_ref,
            x_v, ckv_v, wq_v, wuk_v, wuv_v, wo_v, w1_v, w2_v, c_v, wmod_v,
            wq_w, wuk_w, wuv_w, dup_s, mod_s, q_s, qa_s, s_s, cc_s, ctx_s, y_s,
            small_sems, sems, *, H):
    B, M = x_hbm.shape
    DC = ckv_hbm.shape[1]
    DFF = w1_hbm.shape[1]
    D = LANES
    NP = H // 2
    NK = ckv_hbm.shape[0] // B // KB

    stream = _Stream([
        (wmod_hbm, wmod_v, 32, 8),
        (wq_hbm, wq_v, 2 * WG, 192),
        (wuk_hbm, wuk_v, 2 * WG, 192),
        (ckv_hbm, ckv_v, KB // 4, 48),
        (wuv_hbm, wuv_v, 2 * WG, 192),
        (wo_hbm, wo_v, LANES, 48),
        (w1_hbm, w1_v, 64, 16),
        (w2_hbm, w2_v, LANES, 48),
    ], sems)
    MOD, WQ, WUK, CKV, WUV, WO, W1 = range(7)
    assert all(stream.end(s) - stream.end(s - 1) == H for s in (WQ, WUK, WUV))
    assert (WG // NP) * 8 == LANES and 4 * NK == H

    cp_x = pltpu.make_async_copy(x_hbm, x_v, small_sems.at[0])
    cp_c = pltpu.make_async_copy(c_hbm, c_v, small_sems.at[1])
    stream.begin()
    cp_c.start()
    cp_x.start()

    col = lax.broadcasted_iota(jnp.int32, dup_s.shape, 1) >> 1
    dup_s[...] = (lax.broadcasted_iota(jnp.int32, dup_s.shape, 0)
                  == (col & 7) * (WG // NP) + (col >> 3)).astype(F32).astype(BF16)

    for w32 in (wq_w, wuk_w, wuv_w):
        for g in range(H):
            w32[g * WPITCH + WG:(g + 1) * WPITCH, :] = jnp.zeros((WPITCH - WG, D), U32)
        w32[H * WPITCH:, :] = jnp.zeros((WPITCH, D), U32)
    qa_s[:, H * B:, :] = jnp.zeros((qa_s.shape[0], B, LANES), F32)
    cc_s[...] = jnp.zeros(cc_s.shape, F32)

    def duplicate(x):
        return jnp.concatenate(
            [jnp.dot(t, dup_s[...], preferred_element_type=F32)
             for t in _lane_blocks(x.astype(BF16), LANES)], axis=1)

    def own_head(x):
        row = lax.broadcasted_iota(jnp.int32, x.shape, 0)
        lane = lax.broadcasted_iota(jnp.int32, x.shape, 1)
        return jnp.where((row >= B) == ((lane & 1) == 1), x, 0.0)

    stream.pump_until(stream.end(MOD))
    cp_c.wait()
    cp_x.wait()
    c = c_v[...].astype(F32)
    sc = (c * jax.nn.sigmoid(c)).astype(BF16)
    pump = stream.pumps(12)

    @pl.loop(0, 6)
    def _(i):
        w = wmod_v[:, pl.ds(pl.multiple_of(i * M, M), M)]
        mod_s[i] = jnp.dot(sc, w, preferred_element_type=F32)
        pump(2 * i)
        pump(2 * i + 1)

    h = _layernorm(x_v[...].astype(F32)) * (1.0 + mod_s[1]) + mod_s[0]
    stream.pump_until(stream.done + 1)
    hd = duplicate(h)
    hd = own_head(jnp.concatenate([hd, hd], axis=0)).astype(BF16)

    stream.pump_until(stream.end(WQ) - NP)
    pump = stream.pumps(NP)

    @pl.loop(0, NP)
    def _(j):
        pump(j)
        _to_words(wq_w, wq_v, 2 * j)
        _to_words(wq_w, wq_v, 2 * j + 1)

    assert stream.done == stream.end(WQ)
    pump = stream.pumps(H)

    @pl.loop(0, NP)
    def _(j):
        q_s[j] = jnp.dot(hd, _head_pair(wq_w, j, M, NP), preferred_element_type=F32)
        for g in (2 * j, 2 * j + 1):
            pump(g)
            _to_words(wuk_w, wuk_v, g)

    pump = stream.pumps(H)

    @pl.loop(0, NP)
    def _(j):
        qa = lax.dot_general(q_s[j].astype(BF16), _head_pair(wuk_w, j, DC, NP), _NT,
                             preferred_element_type=F32)
        row = pl.multiple_of(j * 2 * B, 2 * B)
        for i, t in enumerate(_lane_blocks(own_head(qa * (D ** -0.5)), LANES)):
            qa_s[i, pl.ds(row, 2 * B), :] = t
        pump(2 * j)
        pump(2 * j + 1)

    def keys(b, k, part=0, parts=1):
        n = KB // parts
        return ckv_v[pl.ds(pl.multiple_of((b * NK + k) * KB + part * n, n), n), :]

    def fold(op, x):
        return functools.reduce(op, _lane_blocks(x, LANES))

    def queries(b):
        wide = jnp.concatenate(
            [qa_s[i, pl.ds(b, H, stride=B), :] for i in range(qa_s.shape[0])], axis=1)
        return jnp.concatenate(
            [lax.dot_general(t, dup_s[...], _NT, preferred_element_type=F32)
             for t in _lane_blocks(wide.astype(BF16), 2 * LANES)], axis=1).astype(BF16)

    def scores(qa, b, k, part=0, parts=1):
        return lax.dot_general(qa, keys(b, k, part, parts), _NT, preferred_element_type=F32)

    def apply(m, b, k, l, acc):
        p = jnp.exp(s_s[k] - m)
        acc = acc + jnp.dot(p.astype(BF16), keys(b, k), preferred_element_type=F32)
        return l + fold(jnp.add, p), acc

    def finish(b, l, acc):
        cc = duplicate(acc / jnp.sum(l, axis=-1, keepdims=True))
        for i, t in enumerate(_lane_blocks(cc, LANES)):
            cc_s[i, pl.ds(b, H, stride=B), :] = t

    mx0 = jnp.full((H, LANES), -jnp.inf, F32)
    l0 = jnp.zeros((H, LANES), F32)
    acc0 = jnp.zeros((H, DC), F32)

    assert stream.done == stream.end(WUK) + 4 * NK
    qa_first = queries(0)
    wait, start = stream.reserve(2 * NK)

    def first_body(k, mx):
        wait(2 * k)
        start(2 * k)
        s0 = scores(qa_first, 0, k, 0, 2)
        start(2 * k + 1)
        s = jnp.concatenate([s0, scores(qa_first, 0, k, 1, 2)], axis=1)
        s_s[k] = s
        mx = jnp.maximum(mx, fold(jnp.maximum, s))
        wait(2 * k + 1)
        return mx

    mx = lax.fori_loop(0, NK, first_body, mx0)
    wait, start = stream.reserve((B - 1) * 4 * NK)

    def batch_body(b, mx_prev):
        m = jnp.max(mx_prev, axis=-1, keepdims=True)
        qa = queries(b)

        def step(k, carry):
            mx, l, acc = carry
            i = ((b - 1) * NK + k) * 4
            wait(i)
            start(i)
            wait(i + 1)
            start(i + 1)
            s = scores(qa, b, k)
            start(i + 2)
            l, acc = apply(m, b - 1, k, l, acc)
            s_s[k] = s
            mx = jnp.maximum(mx, fold(jnp.maximum, s))
            wait(i + 2)
            wait(i + 3)
            start(i + 3)
            return mx, l, acc

        mx, l, acc = lax.fori_loop(0, NK, step, (mx0, l0, acc0))
        finish(b - 1, l, acc)
        return mx

    mx = lax.fori_loop(1, B, batch_body, mx)
    m_last = jnp.max(mx, axis=-1, keepdims=True)
    pump = stream.pumps(2 * NK)

    def last_body(k, carry):
        carry = apply(m_last, B - 1, k, *carry)
        pump(2 * k)
        for g in range(3):
            _to_words(wuv_w, wuv_v, 4 * k + g)
        pump(2 * k + 1)
        _to_words(wuv_w, wuv_v, 4 * k + 3)
        return carry

    finish(B - 1, *lax.fori_loop(0, NK, last_body, (l0, acc0)))
    assert stream.done == stream.end(WUV)

    stream.pump_until(stream.done + 1)
    pump = stream.pumps(H)

    @pl.loop(0, NP)
    def _(j):
        row = pl.multiple_of(j * 2 * B, 2 * B)
        cc = jnp.concatenate(
            [cc_s[i, pl.ds(row, 2 * B), :] for i in range(cc_s.shape[0])], axis=1)
        ctx_s[j] = jnp.dot(own_head(cc).astype(BF16), _head_pair(wuv_w, j, DC, NP),
                           preferred_element_type=F32)
        pump(2 * j)
        pump(2 * j + 1)

    stream.pump_until(stream.end(WO))
    pump = stream.pumps(H // 8)

    def wo_body(j, attn):
        ctx = jnp.concatenate(
            [ctx_s[4 * j + r, t * B:(t + 1) * B, :] for r in range(4) for t in range(2)], axis=1)
        w = wo_v[pl.ds(pl.multiple_of(j * 8 * D, 8 * D), 8 * D), :]
        attn = attn + jnp.dot(ctx.astype(BF16), w, preferred_element_type=F32)
        pump(j)
        return attn

    attn = lax.fori_loop(0, H // 8, wo_body, jnp.zeros((B, M), F32))

    x1 = x_v[...].astype(F32) + mod_s[2] * attn
    h2 = (_layernorm(x1) * (1.0 + mod_s[4]) + mod_s[3]).astype(BF16)
    stream.pump_until(stream.end(W1))
    f = jnp.maximum(jnp.dot(h2, w1_v[...], preferred_element_type=F32), 0.0).astype(BF16)
    y_s[...] = x1

    def project(lo, hi):
        stream.pump_until(stream.end(W1) + hi)
        return y_s[...] + mod_s[5] * jnp.dot(
            f[:, lo * LANES:hi * LANES], w2_v[lo * LANES:hi * LANES, :],
            preferred_element_type=F32)

    for lo, hi in zip((0,) + W2_CUTS, W2_CUTS):
        y_s[...] = project(lo, hi)
    out_ref[...] = project(W2_CUTS[-1], DFF // LANES).astype(out_ref.dtype)
    assert stream.done == stream.total


@jax.jit
def pallas_adaLN_cond__compressed_kv_cla__dense_activation_relu__decode_kernel(
    A_x: jax.Array,
    A_c_kv: jax.Array,
    A_w_q: jax.Array,
    A_w_uk: jax.Array,
    A_w_uv: jax.Array,
    A_w_o: jax.Array,
    B_x: jax.Array,
    B_w1: jax.Array,
    B_w2: jax.Array,
    c: jax.Array,
    w_mod: jax.Array,
):
    del B_x
    B, SQ, M = A_x.shape
    _, SK, DC = A_c_kv.shape
    _, H, D = A_w_q.shape
    assert SQ == 1 and D == LANES
    operands = (A_x.reshape(B, M), A_c_kv.reshape(B * SK, DC),
                A_w_q.reshape(M * H, D), A_w_uk.reshape(DC * H, D), A_w_uv.reshape(DC * H, D),
                A_w_o.reshape(H * D, M), B_w1, B_w2, c, w_mod)
    words = [pltpu.VMEM(((w.shape[0] // (2 * WG) + 1) * WPITCH, D), U32) for w in operands[2:5]]
    out = pl.pallas_call(
        functools.partial(_kernel, H=H),
        out_shape=jax.ShapeDtypeStruct((B, M), A_x.dtype),
        in_specs=[pl.BlockSpec(memory_space=pltpu.HBM)] * len(operands),
        out_specs=pl.BlockSpec(memory_space=pltpu.VMEM),
        scratch_shapes=[pltpu.VMEM(a.shape, a.dtype) for a in operands] + words + [
            pltpu.VMEM((LANES, 2 * LANES), BF16),
            pltpu.VMEM((6, B, M), F32),
            pltpu.VMEM((H // 2, 2 * B, D), F32),
            pltpu.VMEM((2 * DC // LANES, (H + 1) * B, LANES), F32),
            pltpu.VMEM((SK // KB, H, KB), F32),
            pltpu.VMEM((2 * DC // LANES, (H + 1) * B, LANES), F32),
            pltpu.VMEM((H // 2, 2 * B, D), F32),
            pltpu.VMEM((B, M), F32),
            pltpu.SemaphoreType.DMA((2,)),
            pltpu.SemaphoreType.DMA((RING,)),
        ],
        compiler_params=pltpu.CompilerParams(
            vmem_limit_bytes=100 * 1024 * 1024,
            disable_bounds_checks=True,
            disable_semaphore_checks=True,
        ),
    )(*operands)
    return out.reshape(B, SQ, M)
```
